```python
import jax
import jax.numpy as jnp

def _softmax(x, axis=-1):
    return jax.nn.softmax(x, axis=axis)
def _gelu(x):
    return jax.nn.gelu(x, approximate=True)
def _silu(x):
    return jax.nn.silu(x)
def _sigmoid(x):
    return jax.nn.sigmoid(x)
def _layernorm(x, axis=-1, eps=1e-5):
    m = jnp.mean(x, axis=axis, keepdims=True)
    v = jnp.var(x, axis=axis, keepdims=True)
    return (x - m) / jnp.sqrt(v + eps)
def _scatter_add(tgt, idx, src, axis=0):
    return tgt.at[idx].add(src)
def _segment_sum(src, seg, n):
    return jax.ops.segment_sum(src, seg, n)
class _Rng:
    def __init__(self, key):
        self._k = key
    def _next(self):
        self._k, sub = jax.random.split(self._k)
        return sub
    def normal(self, shape):
        return jax.random.normal(self._next(), shape, dtype=jnp.bfloat16)
    def randint(self, lo, hi, shape):
        return jax.random.randint(self._next(), shape, lo, hi, dtype=jnp.int32)
    def uniform(self, shape, lo=0.0, hi=1.0):
        return jax.random.uniform(self._next(), shape, jnp.bfloat16, lo, hi)
    def permutation(self, n):
        return jax.random.permutation(self._next(), n)


kernel_name = 'interleave_layers__sliding_local_dilated__glu_gated_swiglu__prompt'

def setup_inputs():
    _rng = _Rng(jax.random.key(int.from_bytes(__import__("os").urandom(4), "little")))
    _w = (lambda a: (lambda t: t.astype(jnp.bfloat16) if jnp.issubdtype(t.dtype, jnp.floating) else t)(jnp.asarray(a)))
    def _A_setup():
        B, S, D = 1, 2048, 1024
        return {
            "x": _w((lambda *s: _rng.normal(s) * 0.05)(B, S, D)),
            "wqkv": _w((lambda *s: _rng.normal(s) * 0.05)(D, 3 * D)),
            "wo": _w((lambda *s: _rng.normal(s) * 0.05)(D, D)),
        }
    _A_in = _A_setup()

    def _B_setup():
        B, S, D, F = 1, 2048, 1024, 3584
        return {
            "x": _w((lambda *s: _rng.normal(s) * 0.05)(B, S, D)),
            "w1": _w((lambda *s: _rng.normal(s) * 0.05)(D, F) * (2.0 / D) ** 0.5),
            "w3": _w((lambda *s: _rng.normal(s) * 0.05)(D, F) * (2.0 / D) ** 0.5),
            "w2": _w((lambda *s: _rng.normal(s) * 0.05)(F, D) * (2.0 / F) ** 0.5),
        }
    _B_in = _B_setup()

    return {
        "A_x": _A_in["x"],
        "A_wqkv": _A_in["wqkv"],
        "A_wo": _A_in["wo"],
        "B_x": _B_in["x"],
        "B_w1": _B_in["w1"],
        "B_w3": _B_in["w3"],
        "B_w2": _B_in["w2"],
    }

def reference(A_x, A_wqkv, A_wo, B_x, B_w1, B_w3, B_w2):
    def _A_ref(x, wqkv, wo):
        B, S, D = x.shape
        H = 32; Dh = D // H
        W, dil = 8, 2
        qkv = (lambda x, *d: x.transpose(*d))((x @ wqkv).reshape(B, S, 3, H, Dh), 2, 0, 3, 1, 4)
        q, k, v = qkv[0], qkv[1], qkv[2]
        scale = Dh ** -0.5
        pos = jnp.arange(S)
        off = jnp.arange(W) * dil
        idx = pos[:, None] - off[None, :]
        mask = idx >= 0
        idx_c = jnp.where(mask, idx, 0).reshape(-1)
        kg = k[:, :, idx_c, :].reshape(B, H, S, W, Dh)
        vg = v[:, :, idx_c, :].reshape(B, H, S, W, Dh)
        logits = jnp.einsum("bhsd,bhswd->bhsw", q, kg) * scale
        logits = jnp.where(mask[None, None, :, :], logits, -1e9)
        attn = _softmax(logits, axis=-1)
        o = jnp.einsum("bhsw,bhswd->bhsd", attn, vg)
        return (lambda x, *d: x.transpose(*d))(o, 0, 2, 1, 3).reshape(B, S, D) @ wo

    def _B_ref(x, w1, w3, w2):
        gate = jnp.einsum("bsd,df->bsf", x, w1)
        up = jnp.einsum("bsd,df->bsf", x, w3)
        h = _silu(gate) * up
        out = jnp.einsum("bsf,fd->bsd", h, w2)
        return out

    x = A_x
    x = x + _A_ref(_layernorm(x, axis=-1), A_wqkv, A_wo)
    x = x + _B_ref(_layernorm(x, axis=-1), B_w1, B_w3, B_w2)
    x = x + _A_ref(_layernorm(x, axis=-1), A_wqkv, A_wo)
    x = x + _B_ref(_layernorm(x, axis=-1), B_w1, B_w3, B_w2)
    return x
```

```python
import jax
import jax.numpy as jnp
from jax import lax
import jax.experimental.pallas as pl
import jax.experimental.pallas.tpu as pltpu

CFG = dict(TM=512, FC=512, PITCH=32)
S, D, F, H, DH, W, DIL = 2048, 1024, 3584, 32, 32, 8, 2
HALO = 16
NB = D // 128
F32, BF16 = jnp.float32, jnp.bfloat16


def _ln(x):
    m = jnp.mean(x, axis=-1, keepdims=True)
    c = x - m
    v = jnp.mean(c * c, axis=-1, keepdims=True)
    return (c * lax.rsqrt(v + 1e-5)).astype(BF16)


def _kernel(x_ref, wqkv_h, wo_h, w1_h, w3_h, w2_h, o_ref,
            wqkv, wo, w1, w3, w2, tbuf, xs, q_s, k_s, v_s, kh, vh, a_s, sems):
    TM, FC, PITCH = CFG['TM'], CFG['FC'], CFG['PITCH']
    i = pl.program_id(0)
    cps = [pltpu.make_async_copy(s, d, sems.at[n]) for n, (s, d) in enumerate(
        [(wqkv_h, wqkv), (wo_h, wo), (w1_h, w1), (w3_h, w3), (w2_h, w2)])]

    @pl.when(i == 0)
    def _():
        for c in cps:
            c.start()
        cps[0].wait()

        def perm_rows(t):
            if PITCH == 32:
                tbuf[pl.ds(0, D), :] = t
            else:
                for h in range(H):
                    tbuf[pl.ds(h * PITCH, DH), :] = t[h * DH:(h + 1) * DH]
            return jnp.concatenate([tbuf[pl.ds(d, H, stride=PITCH), :] for d in range(DH)], axis=0)

        def pq(n, c):
            r = pl.multiple_of((n % 8) * 128, 128)
            cc = pl.multiple_of((n // 8) * D, D)
            t = wqkv[pl.ds(r, 128), pl.ds(cc, D)].astype(F32).T
            wqkv[pl.ds(r, 128), pl.ds(cc, D)] = perm_rows(t).T.astype(BF16)
            return c
        lax.fori_loop(0, 24, pq, 0)
        cps[1].wait()

        def po(n, c):
            cc = pl.multiple_of(n * 128, 128)
            wo[:, pl.ds(cc, 128)] = perm_rows(wo[:, pl.ds(cc, 128)].astype(F32)).astype(BF16)
            return c
        lax.fori_loop(0, NB, po, 0)
        for c in cps[2:]:
            c.wait()

    xs[...] = x_ref[...].astype(F32)

    def pair(l, carry):
        xn = _ln(xs[...])
        q_s[...] = jnp.dot(xn, wqkv[:, 0:D], preferred_element_type=F32)
        kk = jnp.dot(xn, wqkv[:, D:2 * D], preferred_element_type=F32)
        for j in range(NB):
            k_s[j, pl.ds(HALO, TM), :] = kk[:, j * 128:(j + 1) * 128]
        vv = jnp.dot(xn, wqkv[:, 2 * D:3 * D], preferred_element_type=F32)
        for j in range(NB):
            v_s[j, pl.ds(HALO, TM), :] = vv[:, j * 128:(j + 1) * 128]

        @pl.when(i == 0)
        def _():
            for j in range(NB):
                k_s[j, pl.ds(0, HALO), :] = jnp.broadcast_to(k_s[j, pl.ds(HALO, 1), :], (HALO, 128))
                v_s[j, pl.ds(0, HALO), :] = jnp.broadcast_to(v_s[j, pl.ds(HALO, 1), :], (HALO, 128))

        @pl.when(i > 0)
        def _():
            k_s[:, pl.ds(0, HALO), :] = kh[l]
            v_s[:, pl.ds(0, HALO), :] = vh[l]
        kh[l] = k_s[:, pl.ds(TM, HALO), :]
        vh[l] = v_s[:, pl.ds(TM, HALO), :]

        def att(g, c):
            r = pl.multiple_of(g * 16, 16)
            pos = i * TM + r + lax.broadcasted_iota(jnp.int32, (16, 128), 0)
            qs = [q_s[pl.ds(r, 16), j * 128:(j + 1) * 128] for j in range(NB)]
            ls = []
            for w in range(W):
                a = None
                for j in range(NB):
                    t = qs[j] * k_s[j, pl.ds(r + (HALO - DIL * w), 16), :]
                    a = t if a is None else a + t
                a = a + pltpu.roll(a, 64, 1)
                a = a + pltpu.roll(a, 32, 1)
                a = a * (DH ** -0.5)
                if w > 0:
                    a = jnp.where(pos >= DIL * w, a, -1e9)
                ls.append(a)
            m = ls[0]
            for w in range(1, W):
                m = jnp.maximum(m, ls[w])
            ps = [jnp.exp(a - m) for a in ls]
            den = ps[0]
            for w in range(1, W):
                den = den + ps[w]
            inv = 1.0 / den
            ps = [p * inv for p in ps]
            for j in range(NB):
                a = None
                for w in range(W):
                    t = ps[w] * v_s[j, pl.ds(r + (HALO - DIL * w), 16), :]
                    a = t if a is None else a + t
                a_s[pl.ds(r, 16), j * 128:(j + 1) * 128] = a.astype(BF16)
            return c
        lax.fori_loop(0, TM // 16, att, 0)

        xs[...] += jnp.dot(a_s[...], wo[...], preferred_element_type=F32)
        xn2 = _ln(xs[...])
        for c in range(F // FC):
            g = jnp.dot(xn2, w1[:, c * FC:(c + 1) * FC], preferred_element_type=F32)
            u = jnp.dot(xn2, w3[:, c * FC:(c + 1) * FC], preferred_element_type=F32)
            h = (g * jax.nn.sigmoid(g) * u).astype(BF16)
            xs[...] += jnp.dot(h, w2[c * FC:(c + 1) * FC, :], preferred_element_type=F32)
        return carry
    lax.fori_loop(0, 2, pair, 0)
    o_ref[...] = xs[...].astype(o_ref.dtype)


@jax.jit
def pallas_interleave_layers__sliding_local_dilated__glu_gated_swiglu__prompt_kernel(A_x, A_wqkv, A_wo, B_x, B_w1, B_w3, B_w2):
    TM = CFG['TM']
    x2 = A_x.reshape(S, D)
    anyspec = pl.BlockSpec(memory_space=pl.ANY)
    out = pl.pallas_call(
        _kernel,
        grid=(S // TM,),
        in_specs=[pl.BlockSpec((TM, D), lambda i: (i, 0))] + [anyspec] * 5,
        out_specs=pl.BlockSpec((TM, D), lambda i: (i, 0)),
        out_shape=jax.ShapeDtypeStruct((S, D), A_x.dtype),
        scratch_shapes=[
            pltpu.VMEM((D, 3 * D), BF16), pltpu.VMEM((D, D), BF16),
            pltpu.VMEM((D, F), BF16), pltpu.VMEM((D, F), BF16), pltpu.VMEM((F, D), BF16),
            pltpu.VMEM((H * 40, 128), F32),
            pltpu.VMEM((TM, D), F32), pltpu.VMEM((TM, D), F32),
            pltpu.VMEM((NB, HALO + TM, 128), F32), pltpu.VMEM((NB, HALO + TM, 128), F32),
            pltpu.VMEM((2, NB, HALO, 128), F32), pltpu.VMEM((2, NB, HALO, 128), F32),
            pltpu.VMEM((TM, D), BF16),
            pltpu.SemaphoreType.DMA((5,)),
        ],
        compiler_params=pltpu.CompilerParams(dimension_semantics=("arbitrary",), vmem_limit_bytes=100 * 1024 * 1024),
    )(x2, A_wqkv, A_wo, B_w1, B_w3, B_w2)
    return out.reshape(1, S, D)
```

```python
import jax
import jax.numpy as jnp
from jax import lax
import jax.experimental.pallas as pl
import jax.experimental.pallas.tpu as pltpu

CFG = dict(FC=512, PITCH=32, KC=256, VC=256, NL=2)
S, D, F, H, DH, W, DIL = 2048, 1024, 3584, 32, 32, 8, 2
TM = 256
NT = S // TM
G = TM // 8
HG = 16
NB = D // 128
F32, BF16, U32 = jnp.float32, jnp.bfloat16, jnp.uint32
SCALE = DH ** -0.5
LOG2E = 1.4426950408889634


def _dot(a, b):
    return jnp.dot(a, b, preferred_element_type=F32)


def _kernel(x_h, wqkv_h, wo_h, w1_h, w3_h, w2_h, o_h,
            wqkv, wo, w1, w3, w2, xio, xs, xn, stage, tbuf, q_s, k_s, v_s, p_s, a_s, sem_x, sem_w, sem_o):
    FC, PITCH, KC, VC = CFG['FC'], CFG['PITCH'], CFG['KC'], CFG['VC']

    def x_copy(t):
        return pltpu.make_async_copy(x_h.at[pl.ds(t * TM, TM), :], xio.at[t], sem_x.at[t])

    def o_copy(t):
        return pltpu.make_async_copy(xio.at[t], o_h.at[pl.ds(t * TM, TM), :], sem_o.at[t])

    qkv_cp = [pltpu.make_async_copy(wqkv_h.at[:, pl.ds(m * D, D)], wqkv.at[m], sem_w.at[m]) for m in range(3)]
    wo_cp = pltpu.make_async_copy(wo_h, wo, sem_w.at[3])
    ffn_cp = [pltpu.make_async_copy(s, d, sem_w.at[4 + n])
              for n, (s, d) in enumerate([(w1_h, w1), (w3_h, w3), (w2_h, w2)])]
    qkv_cp[0].start()
    x_copy(0).start()
    qkv_cp[1].start()
    qkv_cp[2].start()
    wo_cp.start()
    for t in range(1, NT):
        x_copy(t).start()
    for c in ffn_cp:
        c.start()

    def layernorm_to_xn(t):
        xb = [xs[t, j] for j in range(NB)]
        tot = xb[0]
        for j in range(1, NB):
            tot = tot + xb[j]
        mean = jnp.sum(tot, axis=-1, keepdims=True) * (1.0 / D)
        cb = [b - mean for b in xb]
        sq = cb[0] * cb[0]
        for j in range(1, NB):
            sq = sq + cb[j] * cb[j]
        rstd = lax.rsqrt(jnp.sum(sq, axis=-1, keepdims=True) * (1.0 / D) + 1e-5)
        for j in range(NB):
            xn[:, j * 128:(j + 1) * 128] = (cb[j] * rstd).astype(BF16)

    def load_tile(t):
        x_copy(t).wait()
        for j in range(NB):
            stage[j] = xio[t, :, j * 128:(j + 1) * 128].astype(F32)
        for j in range(NB):
            for g in range(G):
                xs[t, j, g * 8:(g + 1) * 8, :] = stage[j, pl.ds(g, 8, stride=G), :]

    def store_tile(t):
        for j in range(NB):
            rows = [xs[t, j, pl.ds((8 * m % G) * 8 + 8 * m // G, 8, stride=8), :] for m in range(G)]
            xio[t, :, j * 128:(j + 1) * 128] = jnp.concatenate(rows, axis=0).astype(BF16)
        o_copy(t).start()

    def head_major_to_dim_major(t):
        if PITCH == DH:
            tbuf[pl.ds(0, D), :] = t
        else:
            for h in range(H):
                tbuf[pl.ds(h * PITCH, DH), :] = t[h * DH:(h + 1) * DH]
        return jnp.concatenate([tbuf[pl.ds(d, H, stride=PITCH), :] for d in range(DH)], axis=0)

    for m in range(3):
        qkv_cp[m].wait()

        def perm_cols(n, c, m=m):
            r = pl.multiple_of(n * 256, 256)
            t = pltpu.bitcast(wqkv[m, pl.ds(r, 256), :], U32).T
            wqkv[m, pl.ds(r, 256), :] = pltpu.bitcast(head_major_to_dim_major(t).T, BF16)
            return c
        lax.fori_loop(0, D // 256, perm_cols, 0)
    wo_cp.wait()

    def perm_rows(n, c):
        cc = pl.multiple_of(n * 128, 128)
        t = pltpu.bitcast(wo[:, pl.ds(cc, 128)].astype(F32), U32)
        wo[:, pl.ds(cc, 128)] = pltpu.bitcast(head_major_to_dim_major(t), F32).astype(BF16)
        return c
    lax.fori_loop(0, NB, perm_rows, 0)

    load_tile(0)
    layernorm_to_xn(0)

    def project_with_halo(t, dst, m, c0, c1):
        val = _dot(xn[...], wqkv[m, :, c0:c1])
        sub = lax.broadcasted_iota(jnp.int32, (HG * 8, 128), 0) % 8
        for j in range(c0 // 128, c1 // 128):
            new = val[:, j * 128 - c0:(j + 1) * 128 - c0]
            old = dst[j, pl.ds(TM, HG * 8), :]
            prev = jnp.where(t == 0, jnp.broadcast_to(new[0:1, :], (HG * 8, 128)),
                             pltpu.roll(old, HG * 8 - 7, 0))
            dst[j, pl.ds(0, HG * 8), :] = jnp.where(sub == 0, prev, pltpu.roll(new[TM - HG * 8:, :], 1, 0))
            dst[j, pl.ds(HG * 8, TM), :] = new

    def probs(t, g):
        r = g * 8
        qs = [q_s[r:r + 8, j * 128:(j + 1) * 128] for j in range(NB)]
        ls = []
        for w in range(W):
            rk = r + (HG - DIL * w) * 8
            a = qs[0] * k_s[0, rk:rk + 8, :]
            for j in range(1, NB):
                a = a + qs[j] * k_s[j, rk:rk + 8, :]
            a = a + pltpu.roll(a, 64, 1)
            a = a + pltpu.roll(a, 32, 1)
            if g < DIL * w:
                pos = t * TM + g + G * lax.broadcasted_iota(jnp.int32, (8, 128), 0)
                a = jnp.where(pos >= DIL * w, a, -1e9 / SCALE)
            ls.append(a)
        mx = ls[0]
        for w in range(1, W):
            mx = jnp.maximum(mx, ls[w])
        ps = [jnp.exp2((a - mx) * (SCALE * LOG2E)) for a in ls]
        den = ps[0]
        for w in range(1, W):
            den = den + ps[w]
        inv = 1.0 / den
        for w in range(W):
            p_s[w, r:r + 8, :] = ps[w] * inv

    def attn_tile(t, l):
        @pl.when(jnp.logical_and(l == 0, t + 1 < NT))
        def _():
            load_tile(t + 1)

        project_with_halo(t, k_s, 1, 0, D)
        q_s[...] = _dot(xn[...], wqkv[0])
        nv = D // VC
        for c in range(nv):
            project_with_halo(t, v_s, 2, c * VC, (c + 1) * VC)
            for g in range(c * G // nv, (c + 1) * G // nv):
                probs(t, g)
        layernorm_to_xn((t + 1) % NT)
        for c in range(D // KC):
            for j in range(c * KC // 128, (c + 1) * KC // 128):
                for g in range(0, G, 2):
                    r = g * 8
                    a = p_s[0, r:r + 16, :] * v_s[j, r + HG * 8:r + HG * 8 + 16, :]
                    for w in range(1, W):
                        rk = r + (HG - DIL * w) * 8
                        a = a + p_s[w, r:r + 16, :] * v_s[j, rk:rk + 16, :]
                    a_s[r:r + 16, j * 128:(j + 1) * 128] = a.astype(BF16)
            y = _dot(a_s[:, c * KC:(c + 1) * KC], wo[c * KC:(c + 1) * KC, :])
            for j in range(NB):
                xs[t, j] += y[:, j * 128:(j + 1) * 128]
        return l

    def ffn_tile(t, l):
        nc = F // FC
        for c in range(nc):
            gate = _dot(xn[...], w1[:, c * FC:(c + 1) * FC])
            up = _dot(xn[...], w3[:, c * FC:(c + 1) * FC])
            h = (gate * jax.nn.sigmoid(gate) * up).astype(BF16)
            if c == nc - 1:
                layernorm_to_xn((t + 1) % NT)
            y = _dot(h, w2[c * FC:(c + 1) * FC, :])
            for j in range(NB):
                xs[t, j] += y[:, j * 128:(j + 1) * 128]

        @pl.when(l == CFG['NL'] - 1)
        def _():
            store_tile(t)
        return l

    def layer(l, c):
        lax.fori_loop(0, NT, attn_tile, l)

        @pl.when(l == 0)
        def _():
            for cp in ffn_cp:
                cp.wait()
        lax.fori_loop(0, NT, ffn_tile, l)
        return c
    lax.fori_loop(0, CFG['NL'], layer, 0)
    for t in range(NT):
        o_copy(t).wait()


@jax.jit
def pallas_interleave_layers__sliding_local_dilated__glu_gated_swiglu__prompt_kernel(
        A_x, A_wqkv, A_wo, B_x, B_w1, B_w3, B_w2):
    del B_x
    anyspec = pl.BlockSpec(memory_space=pl.ANY)
    out = pl.pallas_call(
        _kernel,
        in_specs=[anyspec] * 6,
        out_specs=anyspec,
        out_shape=jax.ShapeDtypeStruct((S, D), A_x.dtype),
        scratch_shapes=[
            pltpu.VMEM((3, D, D), BF16), pltpu.VMEM((D, D), BF16),
            pltpu.VMEM((D, F), BF16), pltpu.VMEM((D, F), BF16), pltpu.VMEM((F, D), BF16),
            pltpu.VMEM((NT, TM, D), BF16),
            pltpu.VMEM((NT, NB, TM, 128), F32),
            pltpu.VMEM((TM, D), BF16),
            pltpu.VMEM((NB, TM, 128), F32),
            pltpu.VMEM((H * 40, 128), U32),
            pltpu.VMEM((TM, D), F32),
            pltpu.VMEM((NB, HG * 8 + TM, 128), F32),
            pltpu.VMEM((NB, HG * 8 + TM, 128), F32),
            pltpu.VMEM((W, TM, 128), F32),
            pltpu.VMEM((TM, D), BF16),
            pltpu.SemaphoreType.DMA((NT,)), pltpu.SemaphoreType.DMA((7,)), pltpu.SemaphoreType.DMA((NT,)),
        ],
        compiler_params=pltpu.CompilerParams(vmem_limit_bytes=100 * 1024 * 1024),
    )(A_x.reshape(S, D), A_wqkv, A_wo, B_w1, B_w3, B_w2)
    return out.reshape(1, S, D)
```

```python
import jax
import jax.numpy as jnp
from jax import lax
import jax.experimental.pallas as pl
import jax.experimental.pallas.tpu as pltpu

CFG = dict(FC=512, PITCH=33, KC=256, VC=256, NL=2, GN=512, DN=1024, LR=16, QN=512, KN=512, ON=512, LB0=1, LBS=4, PVR=16, PG=None, PIN=1)
S, D, F, H, DH, W, DIL = 2048, 1024, 3584, 32, 32, 8, 2
TM = 256
NT = S // TM
G = TM // 8
HG = 16
NB = D // 128
XP = G + 1
F32, BF16, U32 = jnp.float32, jnp.bfloat16, jnp.uint32
SCALE = DH ** -0.5
LOG2E = 1.4426950408889634


def _dot(a, b):
    return jnp.dot(a, b, preferred_element_type=F32)


def _kernel(x_h, wqkv_h, wo_h, w1_h, w3_h, w2_h, o_h,
            wqkv, wo, w1, w3, w2, xio, xs, xn, tbuf, q_s, k_s, v_s, p_s, a_s, sem_x, sem_w, sem_o):
    FC, PITCH, KC, VC = CFG['FC'], CFG['PITCH'], CFG['KC'], CFG['VC']

    def x_copy(t):
        return pltpu.make_async_copy(x_h.at[pl.ds(t * TM, TM), :], xio.at[t], sem_x.at[t])

    def o_copy(t):
        return pltpu.make_async_copy(xio.at[t], o_h.at[pl.ds(t * TM, TM), :], sem_o.at[t])

    qkv_cp = [pltpu.make_async_copy(wqkv_h.at[:, pl.ds(m * D, D)], wqkv.at[m], sem_w.at[m]) for m in range(3)]
    wo_cp = pltpu.make_async_copy(wo_h, wo, sem_w.at[3])
    ffn_cp = [pltpu.make_async_copy(s, d, sem_w.at[4 + n])
              for n, (s, d) in enumerate([(w1_h, w1), (w3_h, w3), (w2_h, w2)])]
    qkv_cp[0].start()
    x_copy(0).start()
    qkv_cp[1].start()
    qkv_cp[2].start()
    wo_cp.start()
    for t in range(1, NT):
        x_copy(t).start()
    for c in ffn_cp:
        c.start()

    def x_rows(t, j, g0, ng):
        return jnp.concatenate([xs[t, j, pl.ds(g0 + g, 8, stride=XP), :] for g in range(ng)], axis=0)

    def add_to_x(t, j, y):
        for g in range(G):
            xs[t, j, pl.ds(g, 8, stride=XP), :] += y[g * 8:(g + 1) * 8]

    def layernorm(t, dst, g0, ng):
        xb = [x_rows(t, j, g0, ng) for j in range(NB)]
        tot = xb[0]
        for j in range(1, NB):
            tot = tot + xb[j]
        mean = jnp.sum(tot, axis=-1, keepdims=True) * (1.0 / D)
        cb = [b - mean for b in xb]
        sq = cb[0] * cb[0]
        for j in range(1, NB):
            sq = sq + cb[j] * cb[j]
        rstd = lax.rsqrt(jnp.sum(sq, axis=-1, keepdims=True) * (1.0 / D) + 1e-5)
        r0 = g0 * 8 if isinstance(g0, int) else pl.multiple_of(g0 * 8, 16)
        for j in range(NB):
            dst[j, pl.ds(r0, ng * 8), :] = (cb[j] * rstd).astype(BF16)

    def load_tile(t):
        x_copy(t).wait()
        for j in range(NB):
            v = xio[t, :, j * 128:(j + 1) * 128].astype(F32)
            for s in range(8):
                xs[t, j, pl.ds(s * XP, G), :] = v[s * G:(s + 1) * G]

    def store_tile(t):
        for j in range(NB):
            v = jnp.concatenate([xs[t, j, pl.ds(s * XP, G), :] for s in range(8)], axis=0)
            xio[t, :, j * 128:(j + 1) * 128] = v.astype(BF16)
        o_copy(t).start()

    def wide(ref, j0=0, j1=NB):
        return jnp.concatenate([ref[j] for j in range(j0, j1)], axis=1)

    def head_major_to_dim_major(t):
        if PITCH == DH:
            tbuf[pl.ds(0, D), :] = t
        else:
            for h in range(H):
                tbuf[pl.ds(h * PITCH, DH), :] = t[h * DH:(h + 1) * DH]
        return jnp.concatenate([tbuf[pl.ds(d, H, stride=PITCH), :] for d in range(DH)], axis=0)

    for m in range(3):
        qkv_cp[m].wait()

        def perm_cols(n, c, m=m):
            r = pl.multiple_of(n * 256, 256)
            t = pltpu.bitcast(wqkv[m, pl.ds(r, 256), :], U32).T
            wqkv[m, pl.ds(r, 256), :] = pltpu.bitcast(head_major_to_dim_major(t).T, BF16)
            return c
        lax.fori_loop(0, D // 256, perm_cols, 0)
    wo_cp.wait()

    def perm_rows(n, c):
        cc = pl.multiple_of(n * 128, 128)
        t = pltpu.bitcast(wo[:, pl.ds(cc, 128)].astype(F32), U32)
        wo[:, pl.ds(cc, 128)] = pltpu.bitcast(head_major_to_dim_major(t), F32).astype(BF16)
        return c
    lax.fori_loop(0, NB, perm_rows, 0)

    load_tile(0)

    def first_ln(n, c):
        layernorm(0, xn.at[0], n * 8, 8)
        return c
    lax.fori_loop(0, G // 8, first_ln, 0)

    def project_with_halo(t, dst, m, c0, c1):
        val = _dot(wide(xn.at[t % 2]), wqkv[m, :, c0:c1])
        sub = lax.broadcasted_iota(jnp.int32, (HG * 8, 128), 0) % 8
        for j in range(c0 // 128, c1 // 128):
            new = val[:, j * 128 - c0:(j + 1) * 128 - c0]
            old = dst[j, pl.ds(TM, HG * 8), :]
            prev = jnp.where(t == 0, jnp.broadcast_to(new[0:1, :], (HG * 8, 128)),
                             pltpu.roll(old, HG * 8 - 7, 0))
            dst[j, pl.ds(0, HG * 8), :] = jnp.where(sub == 0, prev, pltpu.roll(new[TM - HG * 8:, :], 1, 0))
            dst[j, pl.ds(HG * 8, TM), :] = new

    def probs(t, g):
        r = g * 8
        qs = [q_s[j, r:r + 8, :] for j in range(NB)]
        ls = []
        for w in range(W):
            rk = r + (HG - DIL * w) * 8
            a = qs[0] * k_s[0, rk:rk + 8, :]
            for j in range(1, NB):
                a = a + qs[j] * k_s[j, rk:rk + 8, :]
            a = a + pltpu.roll(a, 64, 1)
            a = a + pltpu.roll(a, 32, 1)
            if g < DIL * w:
                pos = t * TM + g + G * lax.broadcasted_iota(jnp.int32, (8, 128), 0)
                a = jnp.where(pos >= DIL * w, a, -1e9 / SCALE)
            ls.append(a)
        mx = ls[0]
        for w in range(1, W):
            mx = jnp.maximum(mx, ls[w])
        ps = [jnp.exp2((a - mx) * (SCALE * LOG2E)) for a in ls]
        den = ps[0]
        for w in range(1, W):
            den = den + ps[w]
        inv = 1.0 / den
        for w in range(W):
            p_s[w, r:r + 8, :] = ps[w] * inv

    def attn_tile(t, l):
        nt = (t + 1) % NT

        @pl.when(jnp.logical_and(l == 0, t + 1 < NT))
        def _():
            load_tile(t + 1)

        KN, QN, ON, LG, PVR = CFG['KN'], CFG['QN'], CFG['ON'], CFG['LR'] // 8, CFG['PVR']
        ln_todo = list(range(0, G, LG))
        nslots = D // KN + D // QN
        per = -(-len(ln_todo) // nslots)

        def ln_step():
            for _ in range(per):
                if ln_todo:
                    layernorm(nt, xn.at[nt % 2], ln_todo.pop(0), LG)
        for c in range(D // KN):
            project_with_halo(t, k_s, 1, c * KN, (c + 1) * KN)
            ln_step()
        for c in range(D // QN):
            val = _dot(wide(xn.at[t % 2]), wqkv[0, :, c * QN:(c + 1) * QN])
            for j in range(QN // 128):
                q_s[c * QN // 128 + j] = val[:, j * 128:(j + 1) * 128]
            ln_step()
        nv = D // VC
        for c in range(nv):
            project_with_halo(t, v_s, 2, c * VC, (c + 1) * VC)
            for g in range(c * G // nv, (c + 1) * G // nv):
                probs(t, g)

        def pv(j):
            for r in range(0, TM, PVR):
                a = p_s[0, r:r + PVR, :] * v_s[j, r + HG * 8:r + HG * 8 + PVR, :]
                for w in range(1, W):
                    rk = r + (HG - DIL * w) * 8
                    a = a + p_s[w, r:r + PVR, :] * v_s[j, rk:rk + PVR, :]
                a_s[j, r:r + PVR, :] = a.astype(BF16)
        nk = D // KC
        for j in range(KC // 128):
            pv(j)
        for c in range(nk):
            nxt = list(range((c + 1) * KC // 128, (c + 2) * KC // 128)) if c + 1 < nk else []
            for n in range(D // ON):
                y = _dot(wide(a_s, c * KC // 128, (c + 1) * KC // 128), wo[c * KC:(c + 1) * KC, n * ON:(n + 1) * ON])
                for j in range(ON // 128):
                    add_to_x(t, n * ON // 128 + j, y[:, j * 128:(j + 1) * 128])
                for j in nxt[n * len(nxt) * ON // D:(n + 1) * len(nxt) * ON // D]:
                    pv(j)
        return l

    def ffn_tile(t, l):
        nc = F // FC
        nt = (t + 1) % NT
        GN, DN, LG = CFG['GN'], CFG['DN'], CFG['LR'] // 8
        ln_todo = list(range(0, G, LG))
        slot = 0
        for c in range(nc):
            hs = []
            for n in range(FC // GN):
                c0 = c * FC + n * GN
                gate = _dot(wide(xn.at[t % 2]), w1[:, c0:c0 + GN])
                if slot >= CFG['LB0'] and ln_todo:
                    for _ in range(CFG['LBS']):
                        layernorm(nt, xn.at[nt % 2], ln_todo.pop(0), LG)
                slot += 1
                up = _dot(wide(xn.at[t % 2]), w3[:, c0:c0 + GN])
                hs.append((gate * jax.nn.sigmoid(gate) * up).astype(BF16))
            h = jnp.concatenate(hs, axis=1)
            if c == nc - 1:
                assert not ln_todo
            for n in range(D // DN):
                y = _dot(h, w2[c * FC:(c + 1) * FC, n * DN:(n + 1) * DN])
                for j in range(DN // 128):
                    add_to_x(t, n * DN // 128 + j, y[:, j * 128:(j + 1) * 128])

        @pl.when(l == CFG['NL'] - 1)
        def _():
            store_tile(t)
        return l

    def layer(l, c):
        lax.fori_loop(0, NT, attn_tile, l)

        @pl.when(l == 0)
        def _():
            for cp in ffn_cp:
                cp.wait()
        lax.fori_loop(0, NT, ffn_tile, l)
        return c
    lax.fori_loop(0, CFG['NL'], layer, 0)
    for t in range(NT):
        o_copy(t).wait()


@jax.jit
def pallas_interleave_layers__sliding_local_dilated__glu_gated_swiglu__prompt_kernel(
        A_x, A_wqkv, A_wo, B_x, B_w1, B_w3, B_w2):
    del B_x
    anyspec = pl.BlockSpec(memory_space=pl.ANY)
    out = pl.pallas_call(
        _kernel,
        in_specs=[anyspec] * 6,
        out_specs=anyspec,
        out_shape=jax.ShapeDtypeStruct((S, D), A_x.dtype),
        scratch_shapes=[
            pltpu.VMEM((3, D, D), BF16), pltpu.VMEM((D, D), BF16),
            pltpu.VMEM((D, F), BF16), pltpu.VMEM((D, F), BF16), pltpu.VMEM((F, D), BF16),
            pltpu.VMEM((NT, TM, D), BF16),
            pltpu.VMEM((NT, NB, 8 * XP, 128), F32),
            pltpu.VMEM((2, NB, TM, 128), BF16),
            pltpu.VMEM((H * 40, 128), U32),
            pltpu.VMEM((NB, TM, 128), F32),
            pltpu.VMEM((NB, HG * 8 + TM, 128), F32),
            pltpu.VMEM((NB, HG * 8 + TM, 128), F32),
            pltpu.VMEM((W, TM, 128), F32),
            pltpu.VMEM((NB, TM, 128), BF16),
            pltpu.SemaphoreType.DMA((NT,)), pltpu.SemaphoreType.DMA((7,)), pltpu.SemaphoreType.DMA((NT,)),
        ],
        compiler_params=pltpu.CompilerParams(vmem_limit_bytes=100 * 1024 * 1024),
    )(A_x.reshape(S, D), A_wqkv, A_wo, B_w1, B_w3, B_w2)
    return out.reshape(1, S, D)
```

```python
import jax
import jax.numpy as jnp
from jax import lax
import jax.experimental.pallas as pl
import jax.experimental.pallas.tpu as pltpu

CFG = dict(FC=3584, AH=3, PITCH=33, KC=256, VC=256, NL=2, GN=512, DN=1024, LR=16, QN=512, KN=512, ON=512, LB0=1, LBS=4, PVR=16, PG=None, PIN=1)
S, D, F, H, DH, W, DIL = 2048, 1024, 3584, 32, 32, 8, 2
TM = 256
NT = S // TM
G = TM // 8
HG = 16
NB = D // 128
PR = 256
XP = G + 1
F32, BF16, U32 = jnp.float32, jnp.bfloat16, jnp.uint32
SCALE = DH ** -0.5
LOG2E = 1.4426950408889634


def _dot(a, b):
    return jnp.dot(a, b, preferred_element_type=F32)


def _kernel(x_h, wqkv_h, wo_h, w1_h, w3_h, w2_h, o_h,
            wqkv, wo, w1, w3, w2, xio, xs, xn, tbuf, q_s, k_s, v_s, p_s, a_s, sem_x, sem_a, sem_w, sem_o):
    FC, PITCH, KC, VC = CFG['FC'], CFG['PITCH'], CFG['KC'], CFG['VC']

    def x_copy(t):
        return pltpu.make_async_copy(x_h.at[pl.ds(t * TM, TM), :], xio.at[t], sem_x.at[t])

    def o_copy(t):
        return pltpu.make_async_copy(xio.at[t], o_h.at[pl.ds(t * TM, TM), :], sem_o.at[t])

    NR = D // PR

    def qkv_copy(n):
        m, r = n // NR, pl.multiple_of((n % NR) * PR, PR)
        return pltpu.make_async_copy(wqkv_h.at[pl.ds(r, PR), pl.ds(pl.multiple_of(m * D, D), D)],
                                     wqkv.at[m, pl.ds(r, PR), :], sem_a.at[n])

    wo_cp = pltpu.make_async_copy(wo_h, wo, sem_a.at[3 * NR])
    ffn_cp = [pltpu.make_async_copy(s, d, sem_w.at[n])
              for n, (s, d) in enumerate([(w1_h, w1), (w3_h, w3), (w2_h, w2)])]
    qkv_copy(0).start()
    x_copy(0).start()
    AH = CFG['AH']
    for n in range(1, AH):
        qkv_copy(n).start()

    def x_rows(t, j, g0, ng):
        return jnp.concatenate([xs[t, j, pl.ds(g0 + g, 8, stride=XP), :] for g in range(ng)], axis=0)

    def add_to_x(t, j, y):
        for g in range(G):
            xs[t, j, pl.ds(g, 8, stride=XP), :] += y[g * 8:(g + 1) * 8]

    def layernorm(t, dst, g0, ng):
        xb = [x_rows(t, j, g0, ng) for j in range(NB)]
        tot = xb[0]
        for j in range(1, NB):
            tot = tot + xb[j]
        mean = jnp.sum(tot, axis=-1, keepdims=True) * (1.0 / D)
        cb = [b - mean for b in xb]
        sq = cb[0] * cb[0]
        for j in range(1, NB):
            sq = sq + cb[j] * cb[j]
        rstd = lax.rsqrt(jnp.sum(sq, axis=-1, keepdims=True) * (1.0 / D) + 1e-5)
        r0 = g0 * 8 if isinstance(g0, int) else pl.multiple_of(g0 * 8, 16)
        for j in range(NB):
            dst[j, pl.ds(r0, ng * 8), :] = (cb[j] * rstd).astype(BF16)

    def load_tile(t):
        x_copy(t).wait()
        for j in range(NB):
            v = xio[t, :, j * 128:(j + 1) * 128].astype(F32)
            for s in range(8):
                xs[t, j, pl.ds(s * XP, G), :] = v[s * G:(s + 1) * G]

    def store_tile(t):
        for j in range(NB):
            v = jnp.concatenate([xs[t, j, pl.ds(s * XP, G), :] for s in range(8)], axis=0)
            xio[t, :, j * 128:(j + 1) * 128] = v.astype(BF16)
        o_copy(t).start()

    def wide(ref, j0=0, j1=NB):
        return jnp.concatenate([ref[j] for j in range(j0, j1)], axis=1)

    def head_major_to_dim_major(t):
        if PITCH == DH:
            tbuf[pl.ds(0, D), :] = t
        else:
            for h in range(H):
                tbuf[pl.ds(h * PITCH, DH), :] = t[h * DH:(h + 1) * DH]
        return jnp.concatenate([tbuf[pl.ds(d, H, stride=PITCH), :] for d in range(DH)], axis=0)

    def perm_cols(n, c):
        qkv_copy(n).wait()

        @pl.when(n + AH < 3 * NR)
        def _():
            qkv_copy(n + AH).start()

        @pl.when(n + AH == 3 * NR)
        def _():
            wo_cp.start()
        m, r = n // NR, pl.multiple_of((n % NR) * PR, PR)
        t = pltpu.bitcast(wqkv[m, pl.ds(r, PR), :], U32).T
        wqkv[m, pl.ds(r, PR), :] = pltpu.bitcast(head_major_to_dim_major(t).T, BF16)
        return c

    def perm_rows(j, c):
        cols = pl.ds(pl.multiple_of(j * 128, 128), 128)
        t = pltpu.bitcast(wo[:, cols].astype(F32), U32)
        wo[:, cols] = pltpu.bitcast(head_major_to_dim_major(t), F32).astype(BF16)
        return c

    def first_ln(n, c):
        layernorm(0, xn.at[0], n * 8, 8)
        return c

    lax.fori_loop(0, 3 * NR, perm_cols, 0)
    load_tile(0)
    lax.fori_loop(0, G // 8, first_ln, 0)
    wo_cp.wait()
    for t in range(1, NT):
        x_copy(t).start()
    for c in ffn_cp:
        c.start()
    lax.fori_loop(0, NB, perm_rows, 0)

    def project_with_halo(t, dst, m, c0, c1):
        val = _dot(wide(xn.at[t % 2]), wqkv[m, :, c0:c1])
        sub = lax.broadcasted_iota(jnp.int32, (HG * 8, 128), 0) % 8
        for j in range(c0 // 128, c1 // 128):
            new = val[:, j * 128 - c0:(j + 1) * 128 - c0]
            old = dst[j, pl.ds(TM, HG * 8), :]
            prev = jnp.where(t == 0, jnp.broadcast_to(new[0:1, :], (HG * 8, 128)),
                             pltpu.roll(old, HG * 8 - 7, 0))
            dst[j, pl.ds(0, HG * 8), :] = jnp.where(sub == 0, prev, pltpu.roll(new[TM - HG * 8:, :], 1, 0))
            dst[j, pl.ds(HG * 8, TM), :] = new

    def probs(t, g):
        r = g * 8
        qs = [q_s[j, r:r + 8, :] for j in range(NB)]
        ls = []
        for w in range(W):
            rk = r + (HG - DIL * w) * 8
            a = qs[0] * k_s[0, rk:rk + 8, :]
            for j in range(1, NB):
                a = a + qs[j] * k_s[j, rk:rk + 8, :]
            a = a + pltpu.roll(a, 64, 1)
            a = a + pltpu.roll(a, 32, 1)
            if g < DIL * w:
                pos = t * TM + g + G * lax.broadcasted_iota(jnp.int32, (8, 128), 0)
                a = jnp.where(pos >= DIL * w, a, -1e9 / SCALE)
            ls.append(a)
        mx = ls[0]
        for w in range(1, W):
            mx = jnp.maximum(mx, ls[w])
        ps = [jnp.exp2((a - mx) * (SCALE * LOG2E)) for a in ls]
        den = ps[0]
        for w in range(1, W):
            den = den + ps[w]
        inv = 1.0 / den
        for w in range(W):
            p_s[w, r:r + 8, :] = ps[w] * inv

    def attn_tile(t, l):
        nt = (t + 1) % NT

        @pl.when(jnp.logical_and(l == 0, t + 1 < NT))
        def _():
            load_tile(t + 1)

        KN, QN, ON, LG, PVR = CFG['KN'], CFG['QN'], CFG['ON'], CFG['LR'] // 8, CFG['PVR']
        ln_todo = list(range(0, G, LG))
        nslots = D // KN + D // QN
        per = -(-len(ln_todo) // nslots)

        def ln_step():
            for _ in range(per):
                if ln_todo:
                    layernorm(nt, xn.at[nt % 2], ln_todo.pop(0), LG)
        for c in range(D // KN):
            project_with_halo(t, k_s, 1, c * KN, (c + 1) * KN)
            ln_step()
        for c in range(D // QN):
            val = _dot(wide(xn.at[t % 2]), wqkv[0, :, c * QN:(c + 1) * QN])
            for j in range(QN // 128):
                q_s[c * QN // 128 + j] = val[:, j * 128:(j + 1) * 128]
            ln_step()
        nv = D // VC
        for c in range(nv):
            project_with_halo(t, v_s, 2, c * VC, (c + 1) * VC)
            for g in range(c * G // nv, (c + 1) * G // nv):
                probs(t, g)

        def pv(j):
            for r in range(0, TM, PVR):
                a = p_s[0, r:r + PVR, :] * v_s[j, r + HG * 8:r + HG * 8 + PVR, :]
                for w in range(1, W):
                    rk = r + (HG - DIL * w) * 8
                    a = a + p_s[w, r:r + PVR, :] * v_s[j, rk:rk + PVR, :]
                a_s[j, r:r + PVR, :] = a.astype(BF16)
        nk = D // KC
        for j in range(KC // 128):
            pv(j)
        for c in range(nk):
            nxt = list(range((c + 1) * KC // 128, (c + 2) * KC // 128)) if c + 1 < nk else []
            for n in range(D // ON):
                y = _dot(wide(a_s, c * KC // 128, (c + 1) * KC // 128), wo[c * KC:(c + 1) * KC, n * ON:(n + 1) * ON])
                for j in range(ON // 128):
                    add_to_x(t, n * ON // 128 + j, y[:, j * 128:(j + 1) * 128])
                for j in nxt[n * len(nxt) * ON // D:(n + 1) * len(nxt) * ON // D]:
                    pv(j)
        return l

    def ffn_tile(t, l):
        nc = F // FC
        nt = (t + 1) % NT
        GN, DN, LG = CFG['GN'], CFG['DN'], CFG['LR'] // 8
        ln_todo = list(range(0, G, LG))
        slot = 0
        for c in range(nc):
            hs = []
            for n in range(FC // GN):
                c0 = c * FC + n * GN
                gate = _dot(wide(xn.at[t % 2]), w1[:, c0:c0 + GN])
                if slot >= CFG['LB0'] and ln_todo:
                    for _ in range(CFG['LBS']):
                        layernorm(nt, xn.at[nt % 2], ln_todo.pop(0), LG)
                slot += 1
                up = _dot(wide(xn.at[t % 2]), w3[:, c0:c0 + GN])
                hs.append((gate * jax.nn.sigmoid(gate) * up).astype(BF16))
            h = jnp.concatenate(hs, axis=1)
            if c == nc - 1:
                assert not ln_todo
            for n in range(D // DN):
                y = _dot(h, w2[c * FC:(c + 1) * FC, n * DN:(n + 1) * DN])
                for j in range(DN // 128):
                    add_to_x(t, n * DN // 128 + j, y[:, j * 128:(j + 1) * 128])

        @pl.when(l == CFG['NL'] - 1)
        def _():
            store_tile(t)
        return l

    def layer(l, c):
        lax.fori_loop(0, NT, attn_tile, l)

        @pl.when(l == 0)
        def _():
            for cp in ffn_cp:
                cp.wait()
        lax.fori_loop(0, NT, ffn_tile, l)
        return c
    if CFG['NL'] == 0:
        for c in [x_copy(t) for t in range(1, NT)] + ffn_cp:
            c.wait()
        return
    lax.fori_loop(0, CFG['NL'], layer, 0)
    for t in range(NT):
        o_copy(t).wait()


@jax.jit
def pallas_interleave_layers__sliding_local_dilated__glu_gated_swiglu__prompt_kernel(
        A_x, A_wqkv, A_wo, B_x, B_w1, B_w3, B_w2):
    del B_x
    anyspec = pl.BlockSpec(memory_space=pl.ANY)
    out = pl.pallas_call(
        _kernel,
        in_specs=[anyspec] * 6,
        out_specs=anyspec,
        out_shape=jax.ShapeDtypeStruct((S, D), A_x.dtype),
        scratch_shapes=[
            pltpu.VMEM((3, D, D), BF16), pltpu.VMEM((D, D), BF16),
            pltpu.VMEM((D, F), BF16), pltpu.VMEM((D, F), BF16), pltpu.VMEM((F, D), BF16),
            pltpu.VMEM((NT, TM, D), BF16),
            pltpu.VMEM((NT, NB, 8 * XP, 128), F32),
            pltpu.VMEM((2, NB, TM, 128), BF16),
            pltpu.VMEM((H * 40, 128), U32),
            pltpu.VMEM((NB, TM, 128), F32),
            pltpu.VMEM((NB, HG * 8 + TM, 128), F32),
            pltpu.VMEM((NB, HG * 8 + TM, 128), F32),
            pltpu.VMEM((W, TM, 128), F32),
            pltpu.VMEM((NB, TM, 128), BF16),
            pltpu.SemaphoreType.DMA((NT,)), pltpu.SemaphoreType.DMA((3 * D // PR + 1,)), pltpu.SemaphoreType.DMA((3,)), pltpu.SemaphoreType.DMA((NT,)),
        ],
        compiler_params=pltpu.CompilerParams(vmem_limit_bytes=100 * 1024 * 1024),
    )(A_x.reshape(S, D), A_wqkv, A_wo, B_w1, B_w3, B_w2)
    return out.reshape(1, S, D)
```

```python
import jax
import jax.numpy as jnp
from jax import lax
import jax.experimental.pallas as pl
import jax.experimental.pallas.tpu as pltpu

CFG = dict(FC=3584, AH=3, PITCH=33, KC=512, VC=512, NL=2, GN=512, DN=1024, LR=16, QN=512, KN=512, ON=512, LB0=1, LBS=4, PVR=16, PG=None, FLAGS=None, QFIRST=0, LNK=1)
S, D, F, H, DH, W, DIL = 2048, 1024, 3584, 32, 32, 8, 2
TM = 256
NT = S // TM
G = TM // 8
HG = 16
NB = D // 128
PR = 256
PITCH = DH + 1
XP = G + 1
F32, BF16, U32 = jnp.float32, jnp.bfloat16, jnp.uint32
SCALE = DH ** -0.5
LOG2E = 1.4426950408889634


def _dot(a, b):
    return jnp.dot(a, b, preferred_element_type=F32)


def _kernel(x_h, wqkv_h, wo_h, w1_h, w3_h, w2_h, o_h,
            wqkv_in, wo_in, wqkv, wo, w1, w3, w2, xio, xs, xn, tbuf, tbuf2, q_s, k_s, v_s, p_s, a_s, sem_x, sem_a, sem_w, sem_o):
    FC, KC, VC = CFG['FC'], CFG['KC'], CFG['VC']

    def x_copy(t):
        return pltpu.make_async_copy(x_h.at[pl.ds(t * TM, TM), :], xio.at[t], sem_x.at[t])

    def o_copy(t):
        return pltpu.make_async_copy(xio.at[t], o_h.at[pl.ds(t * TM, TM), :], sem_o.at[t])

    NR = D // PR

    def qkv_copy(n):
        m, r = n // NR, pl.multiple_of((n % NR) * PR, PR)
        return pltpu.make_async_copy(wqkv_h.at[pl.ds(r, PR), pl.ds(pl.multiple_of(m * D, D), D)],
                                     wqkv_in.at[m, pl.ds(r, PR), :], sem_a.at[n])

    def wo_copy(j):
        return pltpu.make_async_copy(wo_h.at[:, pl.ds(pl.multiple_of(j * 128, 128), 128)], wo_in.at[j],
                                     sem_a.at[3 * NR + j])

    ffn_cp = [pltpu.make_async_copy(s, d, sem_w.at[n])
              for n, (s, d) in enumerate([(w1_h, w1), (w3_h, w3), (w2_h, w2)])]
    AH = CFG['AH']
    for n in range(AH):
        qkv_copy(n).start()
        wo_copy(n).start()

    def x_rows(t, j, g0, ng):
        return jnp.concatenate([xs[t, j, pl.ds(g0 + g, 8, stride=XP), :] for g in range(ng)], axis=0)

    def add_to_x(t, j, y):
        for g in range(G):
            xs[t, j, pl.ds(g, 8, stride=XP), :] += y[g * 8:(g + 1) * 8]

    def layernorm(t, dst, g0, ng):
        xb = [x_rows(t, j, g0, ng) for j in range(NB)]
        tot = xb[0]
        for j in range(1, NB):
            tot = tot + xb[j]
        mean = jnp.sum(tot, axis=-1, keepdims=True) * (1.0 / D)
        cb = [b - mean for b in xb]
        sq = cb[0] * cb[0]
        for j in range(1, NB):
            sq = sq + cb[j] * cb[j]
        rstd = lax.rsqrt(jnp.sum(sq, axis=-1, keepdims=True) * (1.0 / D) + 1e-5)
        r0 = g0 * 8 if isinstance(g0, int) else pl.multiple_of(g0 * 8, 16)
        for j in range(NB):
            dst[j, pl.ds(r0, ng * 8), :] = (cb[j] * rstd).astype(BF16)

    def load_tile(t):
        x_copy(t).wait()
        for j in range(NB):
            v = xio[t, :, j * 128:(j + 1) * 128].astype(F32)
            for s in range(8):
                xs[t, j, pl.ds(s * XP, G), :] = v[s * G:(s + 1) * G]

    def store_tile(t):
        for j in range(NB):
            v = jnp.concatenate([xs[t, j, pl.ds(s * XP, G), :] for s in range(8)], axis=0)
            xio[t, :, j * 128:(j + 1) * 128] = v.astype(BF16)
        o_copy(t).start()

    def wide(ref, j0=0, j1=NB):
        return jnp.concatenate([ref[j] for j in range(j0, j1)], axis=1)

    def head_major_to_dim_major(t, buf):
        for h in range(H):
            buf[pl.ds(h * PITCH, DH), :] = t[h * DH:(h + 1) * DH]
        return jnp.concatenate([buf[pl.ds(d, H, stride=PITCH), :] for d in range(DH)], axis=0)

    def prefetch(n):
        @pl.when(n < 3 * NR)
        def _():
            qkv_copy(n).start()

        @pl.when(n < NB)
        def _():
            wo_copy(n).start()

        @pl.when(n == NB)
        def _():
            x_copy(0).start()

    def perm_cols(n):
        m, r = n // NR, pl.multiple_of((n % NR) * PR, PR)
        t = pltpu.bitcast(wqkv_in[m, pl.ds(r, PR), :], U32).T
        wp = pltpu.bitcast(head_major_to_dim_major(t, tbuf).T, BF16)
        for j in range(NB):
            wqkv[m, j, pl.ds(r, PR), :] = wp[:, j * 128:(j + 1) * 128]

    def prologue_a(n, c):
        qkv_copy(n).wait()
        wo_copy(n).wait()
        prefetch(n + AH)
        perm_cols(n)
        t = pltpu.bitcast(wo_in[n].astype(F32), U32)
        wo[n] = pltpu.bitcast(head_major_to_dim_major(t, tbuf2), F32).astype(BF16)
        return c

    def prologue_b(n, c):
        qkv_copy(n).wait()
        prefetch(n + AH)
        perm_cols(n)
        ng = G // (3 * NR - NB)
        layernorm(0, xn.at[0], (n - NB) * ng, ng)
        return c

    lax.fori_loop(0, NB, prologue_a, 0)
    load_tile(0)
    lax.fori_loop(NB, 3 * NR, prologue_b, 0)
    for t in range(1, NT):
        x_copy(t).start()
    for c in ffn_cp:
        c.start()

    def project_with_halo(t, dst, m, c0, c1):
        val = _dot(wide(xn.at[t % 2]), wide(wqkv.at[m], c0 // 128, c1 // 128))
        sub = lax.broadcasted_iota(jnp.int32, (HG * 8, 128), 0) % 8
        for j in range(c0 // 128, c1 // 128):
            new = val[:, j * 128 - c0:(j + 1) * 128 - c0]
            old = dst[j, pl.ds(TM, HG * 8), :]
            prev = jnp.where(t == 0, jnp.broadcast_to(new[0:1, :], (HG * 8, 128)),
                             pltpu.roll(old, HG * 8 - 7, 0))
            dst[j, pl.ds(0, HG * 8), :] = jnp.where(sub == 0, prev, pltpu.roll(new[TM - HG * 8:, :], 1, 0))
            dst[j, pl.ds(HG * 8, TM), :] = new

    def probs(t, g):
        r = g * 8
        qs = [q_s[j, r:r + 8, :] for j in range(NB)]
        ls = []
        for w in range(W):
            rk = r + (HG - DIL * w) * 8
            a = qs[0] * k_s[0, rk:rk + 8, :]
            for j in range(1, NB):
                a = a + qs[j] * k_s[j, rk:rk + 8, :]
            a = a + pltpu.roll(a, 64, 1)
            a = a + pltpu.roll(a, 32, 1)
            if g < DIL * w:
                pos = t * TM + g + G * lax.broadcasted_iota(jnp.int32, (8, 128), 0)
                a = jnp.where(pos >= DIL * w, a, -1e9 / SCALE)
            ls.append(a)
        mx = ls[0]
        for w in range(1, W):
            mx = jnp.maximum(mx, ls[w])
        ps = [jnp.exp2((a - mx) * (SCALE * LOG2E)) for a in ls]
        den = ps[0]
        for w in range(1, W):
            den = den + ps[w]
        inv = 1.0 / den
        for w in range(W):
            p_s[w, r:r + 8, :] = ps[w] * inv

    def attn_tile(t, l):
        nt = (t + 1) % NT

        @pl.when(jnp.logical_and(l == 0, t + 1 < NT))
        def _():
            load_tile(t + 1)

        KN, QN, ON, LG, PVR = CFG['KN'], CFG['QN'], CFG['ON'], CFG['LR'] // 8, CFG['PVR']
        ln_todo = list(range(0, G, LG))
        nslots = D // KN + D // QN
        per = -(-len(ln_todo) * CFG['LNK'] // nslots)

        def ln_step():
            for _ in range(per):
                if ln_todo:
                    layernorm(nt, xn.at[nt % 2], ln_todo.pop(0), LG)
        def kproj(c):
            project_with_halo(t, k_s, 1, c * KN, (c + 1) * KN)

        def qproj(c):
            val = _dot(wide(xn.at[t % 2]), wide(wqkv.at[0], c * QN // 128, (c + 1) * QN // 128))
            for j in range(QN // 128):
                q_s[c * QN // 128 + j] = val[:, j * 128:(j + 1) * 128]
        ks = [(kproj, c) for c in range(D // KN)]
        qs = [(qproj, c) for c in range(D // QN)]
        order = {0: ks + qs, 1: qs + ks, 2: [e for pr in zip(ks, qs) for e in pr]}[CFG['QFIRST']]
        for f, c in order:
            f(c)
            ln_step()
        nv = D // VC
        for c in range(nv):
            project_with_halo(t, v_s, 2, c * VC, (c + 1) * VC)
            for g in range(c * G // nv, (c + 1) * G // nv):
                probs(t, g)

        def pv(j):
            for r in range(0, TM, PVR):
                a = p_s[0, r:r + PVR, :] * v_s[j, r + HG * 8:r + HG * 8 + PVR, :]
                for w in range(1, W):
                    rk = r + (HG - DIL * w) * 8
                    a = a + p_s[w, r:r + PVR, :] * v_s[j, rk:rk + PVR, :]
                a_s[j, r:r + PVR, :] = a.astype(BF16)
        nk = D // KC
        for j in range(KC // 128):
            pv(j)
        for c in range(nk):
            nxt = list(range((c + 1) * KC // 128, (c + 2) * KC // 128)) if c + 1 < nk else []
            for n in range(D // ON):
                y = _dot(wide(a_s, c * KC // 128, (c + 1) * KC // 128), wide(wo.at[:, c * KC:(c + 1) * KC, :], n * ON // 128, (n + 1) * ON // 128))
                for j in range(ON // 128):
                    add_to_x(t, n * ON // 128 + j, y[:, j * 128:(j + 1) * 128])
                for j in nxt[n * len(nxt) * ON // D:(n + 1) * len(nxt) * ON // D]:
                    pv(j)
        return l

    def ffn_tile(t, l):
        nc = F // FC
        nt = (t + 1) % NT
        GN, DN, LG = CFG['GN'], CFG['DN'], CFG['LR'] // 8
        ln_todo = list(range(0, G, LG))
        slot = 0
        for c in range(nc):
            hs = []
            for n in range(FC // GN):
                c0 = c * FC + n * GN
                gate = _dot(wide(xn.at[t % 2]), w1[:, c0:c0 + GN])
                if slot >= CFG['LB0'] and ln_todo:
                    for _ in range(CFG['LBS']):
                        layernorm(nt, xn.at[nt % 2], ln_todo.pop(0), LG)
                slot += 1
                up = _dot(wide(xn.at[t % 2]), w3[:, c0:c0 + GN])
                hs.append((gate * jax.nn.sigmoid(gate) * up).astype(BF16))
            h = jnp.concatenate(hs, axis=1)
            if c == nc - 1:
                assert not ln_todo
            for n in range(D // DN):
                y = _dot(h, w2[c * FC:(c + 1) * FC, n * DN:(n + 1) * DN])
                for j in range(DN // 128):
                    add_to_x(t, n * DN // 128 + j, y[:, j * 128:(j + 1) * 128])

        @pl.when(l == CFG['NL'] - 1)
        def _():
            store_tile(t)
        return l

    def layer(l, c):
        lax.fori_loop(0, NT, attn_tile, l)

        @pl.when(l == 0)
        def _():
            for cp in ffn_cp:
                cp.wait()
        lax.fori_loop(0, NT, ffn_tile, l)
        return c
    if CFG['NL'] == 0:
        for c in [x_copy(t) for t in range(1, NT)] + ffn_cp:
            c.wait()
        return
    lax.fori_loop(0, CFG['NL'], layer, 0)
    for t in range(NT):
        o_copy(t).wait()


@jax.jit
def pallas_interleave_layers__sliding_local_dilated__glu_gated_swiglu__prompt_kernel(
        A_x, A_wqkv, A_wo, B_x, B_w1, B_w3, B_w2):
    del B_x
    anyspec = pl.BlockSpec(memory_space=pl.ANY)
    out = pl.pallas_call(
        _kernel,
        in_specs=[anyspec] * 6,
        out_specs=anyspec,
        out_shape=jax.ShapeDtypeStruct((S, D), A_x.dtype),
        scratch_shapes=[
            pltpu.VMEM((3, D, D), BF16), pltpu.VMEM((NB, D, 128), BF16),
            pltpu.VMEM((3, NB, D, 128), BF16), pltpu.VMEM((NB, D, 128), BF16),
            pltpu.VMEM((D, F), BF16), pltpu.VMEM((D, F), BF16), pltpu.VMEM((F, D), BF16),
            pltpu.VMEM((NT, TM, D), BF16),
            pltpu.VMEM((NT, NB, 8 * XP, 128), F32),
            pltpu.VMEM((2, NB, TM, 128), BF16),
            pltpu.VMEM((H * PITCH, 128), U32), pltpu.VMEM((H * PITCH, 128), U32),
            pltpu.VMEM((NB, TM, 128), F32),
            pltpu.VMEM((NB, HG * 8 + TM, 128), F32),
            pltpu.VMEM((NB, HG * 8 + TM, 128), F32),
            pltpu.VMEM((W, TM, 128), F32),
            pltpu.VMEM((NB, TM, 128), BF16),
            pltpu.SemaphoreType.DMA((NT,)), pltpu.SemaphoreType.DMA((3 * D // PR + NB,)), pltpu.SemaphoreType.DMA((3,)), pltpu.SemaphoreType.DMA((NT,)),
        ],
        compiler_params=pltpu.CompilerParams(vmem_limit_bytes=100 * 1024 * 1024, flags=CFG['FLAGS']),
    )(A_x.reshape(S, D), A_wqkv, A_wo, B_w1, B_w3, B_w2)
    return out.reshape(1, S, D)
```

```python
import jax
import jax.numpy as jnp
from jax import lax
import jax.experimental.pallas as pl
import jax.experimental.pallas.tpu as pltpu

S, D, F = 2048, 1024, 3584
H, DH, W, DIL = 32, 32, 8, 2
N_LAYERS = 2
TM = 256
NT = S // TM
G = TM // 8
HG = 16
NB = D // 128
XP = G + 1
PITCH = DH + 1
PR = 256
NR = D // PR
AHEAD = 3
F32, BF16, U32 = jnp.float32, jnp.bfloat16, jnp.uint32
SCALE = DH ** -0.5
LOG2E = 1.4426950408889634


def _dot(a, b):
    return jnp.dot(a, b, preferred_element_type=F32)


def _wide(ref, j0=0, j1=NB):
    return jnp.concatenate([ref[j] for j in range(j0, j1)], axis=1)


def _block(val, j):
    return val[:, j * 128:(j + 1) * 128]


def _head_major_to_dim_major(val, buf):
    for h in range(H):
        buf[pl.ds(h * PITCH, DH), :] = val[h * DH:(h + 1) * DH]
    return jnp.concatenate([buf[pl.ds(d, H, stride=PITCH), :] for d in range(DH)], axis=0)


def _kernel(x_h, wqkv_h, wo_h, w1_h, w3_h, w2_h, o_h,
            wqkv_in, wo_in, wqkv, wo, w1, w3, w2, xio, xs, xn, tbuf_a, tbuf_b,
            q_s, k_s, v_s, p_s, a_s, sem_x, sem_a, sem_w, sem_o):

    def x_copy(t):
        return pltpu.make_async_copy(x_h.at[pl.ds(t * TM, TM), :], xio.at[t], sem_x.at[t])

    def o_copy(t):
        return pltpu.make_async_copy(xio.at[t], o_h.at[pl.ds(t * TM, TM), :], sem_o.at[t])

    def qkv_copy(n):
        m = n // NR
        rows = pl.ds(pl.multiple_of((n % NR) * PR, PR), PR)
        cols = pl.ds(pl.multiple_of(m * D, D), D)
        return pltpu.make_async_copy(wqkv_h.at[rows, cols], wqkv_in.at[m, rows, :], sem_a.at[n])

    def wo_copy(j):
        cols = pl.ds(pl.multiple_of(j * 128, 128), 128)
        return pltpu.make_async_copy(wo_h.at[:, cols], wo_in.at[j], sem_a.at[3 * NR + j])

    ffn_copies = [pltpu.make_async_copy(src, dst, sem_w.at[n])
                  for n, (src, dst) in enumerate([(w1_h, w1), (w3_h, w3), (w2_h, w2)])]

    def x_rows(t, j, g0, ng):
        return jnp.concatenate([xs[t, j, pl.ds(g0 + g, 8, stride=XP), :] for g in range(ng)], axis=0)

    def add_to_x(t, j, y):
        for g in range(G):
            xs[t, j, pl.ds(g, 8, stride=XP), :] += y[g * 8:(g + 1) * 8]

    def load_tile(t):
        x_copy(t).wait()
        for j in range(NB):
            val = xio[t, :, j * 128:(j + 1) * 128].astype(F32)
            for s in range(8):
                xs[t, j, pl.ds(s * XP, G), :] = val[s * G:(s + 1) * G]

    def store_tile(t):
        for j in range(NB):
            val = jnp.concatenate([xs[t, j, pl.ds(s * XP, G), :] for s in range(8)], axis=0)
            xio[t, :, j * 128:(j + 1) * 128] = val.astype(BF16)
        o_copy(t).start()

    def layernorm(t, dst, g0, ng):
        xb = [x_rows(t, j, g0, ng) for j in range(NB)]
        tot = xb[0]
        for j in range(1, NB):
            tot = tot + xb[j]
        mean = jnp.sum(tot, axis=-1, keepdims=True) * (1.0 / D)
        cb = [b - mean for b in xb]
        sq = cb[0] * cb[0]
        for j in range(1, NB):
            sq = sq + cb[j] * cb[j]
        rstd = lax.rsqrt(jnp.sum(sq, axis=-1, keepdims=True) * (1.0 / D) + 1e-5)
        r0 = g0 * 8 if isinstance(g0, int) else pl.multiple_of(g0 * 8, 16)
        for j in range(NB):
            dst[j, pl.ds(r0, ng * 8), :] = (cb[j] * rstd).astype(BF16)

    def next_tile_layernorm(t):
        nt = (t + 1) % NT
        todo = list(range(0, G, 2))

        def step(n):
            for _ in range(min(n, len(todo))):
                layernorm(nt, xn.at[nt % 2], todo.pop(0), 2)
        return step, todo

    def prefetch(n):
        @pl.when(n < 3 * NR)
        def _():
            qkv_copy(n).start()

        @pl.when(n < NB)
        def _():
            wo_copy(n).start()

        @pl.when(n == NB)
        def _():
            x_copy(0).start()

    def reorder_qkv_columns(n):
        m = n // NR
        rows = pl.ds(pl.multiple_of((n % NR) * PR, PR), PR)
        t = pltpu.bitcast(wqkv_in[m, rows, :], U32).T
        val = pltpu.bitcast(_head_major_to_dim_major(t, tbuf_a).T, BF16)
        for j in range(NB):
            wqkv[m, j, rows, :] = _block(val, j)

    def prologue_a(n, carry):
        qkv_copy(n).wait()
        wo_copy(n).wait()
        prefetch(n + AHEAD)
        reorder_qkv_columns(n)
        t = pltpu.bitcast(wo_in[n].astype(F32), U32)
        wo[n] = pltpu.bitcast(_head_major_to_dim_major(t, tbuf_b), F32).astype(BF16)
        k_s[n, pl.ds(TM, HG * 8), :] = jnp.zeros((HG * 8, 128), F32)
        v_s[n, pl.ds(TM, HG * 8), :] = jnp.zeros((HG * 8, 128), F32)
        return carry

    def prologue_b(n, carry):
        qkv_copy(n).wait()
        prefetch(n + AHEAD)
        reorder_qkv_columns(n)
        ng = G // (3 * NR - NB)
        layernorm(0, xn.at[0], (n - NB) * ng, ng)
        return carry

    for n in range(AHEAD):
        qkv_copy(n).start()
        wo_copy(n).start()
    lax.fori_loop(0, NB, prologue_a, 0)
    load_tile(0)
    lax.fori_loop(NB, 3 * NR, prologue_b, 0)
    for t in range(1, NT):
        x_copy(t).start()
    for c in ffn_copies:
        c.start()

    def project_with_halo(t, dst, m, j0, j1):
        val = _dot(_wide(xn.at[t % 2]), _wide(wqkv.at[m], j0, j1))
        sub = lax.broadcasted_iota(jnp.int32, (HG * 8, 128), 0) % 8
        for j in range(j0, j1):
            new = _block(val, j - j0)
            old = dst[j, pl.ds(TM, HG * 8), :]
            prev = jnp.where(t == 0, jnp.broadcast_to(new[0:1, :], (HG * 8, 128)),
                             pltpu.roll(old, HG * 8 - 7, 0))
            dst[j, pl.ds(0, HG * 8), :] = jnp.where(sub == 0, prev, pltpu.roll(new[TM - HG * 8:, :], 1, 0))
            dst[j, pl.ds(HG * 8, TM), :] = new

    def softmax_weights(t, g):
        r = g * 8
        qs = [q_s[j, r:r + 8, :] for j in range(NB)]
        logits = []
        for w in range(W):
            rk = r + (HG - DIL * w) * 8
            a = qs[0] * k_s[0, rk:rk + 8, :]
            for j in range(1, NB):
                a = a + qs[j] * k_s[j, rk:rk + 8, :]
            a = (a + pltpu.roll(a, 64, 1)) + (pltpu.roll(a, 32, 1) + pltpu.roll(a, 96, 1))
            if g < DIL * w:
                pos = t * TM + g + G * lax.broadcasted_iota(jnp.int32, (8, 128), 0)
                a = jnp.where(pos >= DIL * w, a, -1e9 / SCALE)
            logits.append(a)
        mx = logits[0]
        for w in range(1, W):
            mx = jnp.maximum(mx, logits[w])
        ps = [jnp.exp2((a - mx) * (SCALE * LOG2E)) for a in logits]
        den = ps[0]
        for w in range(1, W):
            den = den + ps[w]
        for w in range(W):
            p_s[w, r:r + 8, :] = ps[w]
        p_s[W, r:r + 8, :] = 1.0 / den

    def weighted_values(j):
        for r in range(0, TM, 16):
            a = p_s[0, r:r + 16, :] * v_s[j, r + HG * 8:r + HG * 8 + 16, :]
            for w in range(1, W):
                rk = r + (HG - DIL * w) * 8
                a = a + p_s[w, r:r + 16, :] * v_s[j, rk:rk + 16, :]
            a_s[j, r:r + 16, :] = (a * p_s[W, r:r + 16, :]).astype(BF16)

    def attention_tile(t, layer):
        @pl.when(jnp.logical_and(layer == 0, t + 1 < NT))
        def _():
            load_tile(t + 1)

        ln_step, ln_todo = next_tile_layernorm(t)
        for j in range(0, NB, 2):
            project_with_halo(t, k_s, 1, j, j + 2)
            ln_step(3)
        for r in range(0, TM, TM // 2):
            val = _dot(_wide(xn.at[t % 2, :, r:r + TM // 2, :]), _wide(wqkv.at[0]))
            for j in range(NB):
                q_s[j, r:r + TM // 2, :] = _block(val, j)
            ln_step(3)
        assert not ln_todo
        hb = NB // 2
        for c in range(2):
            project_with_halo(t, v_s, 2, c * hb, (c + 1) * hb)
            for g in range(c * G // 2, (c + 1) * G // 2):
                softmax_weights(t, g)
        for j in range(hb):
            weighted_values(j)
        for c in range(2):
            for n in range(2):
                y = _dot(_wide(a_s, c * hb, (c + 1) * hb),
                         _wide(wo.at[:, c * hb * 128:(c + 1) * hb * 128, :], n * hb, (n + 1) * hb))
                for j in range(hb):
                    add_to_x(t, n * hb + j, _block(y, j))
                if c == 0:
                    for j in range(hb + n * hb // 2, hb + (n + 1) * hb // 2):
                        weighted_values(j)
        return layer

    def ffn_tile(t, layer):
        ln_step, ln_todo = next_tile_layernorm(t)
        hs = []
        for n in range(F // 128):
            gate = _dot(_wide(xn.at[t % 2]), w1[:, n * 128:(n + 1) * 128])
            if n >= 4:
                ln_step(1)
            up = _dot(_wide(xn.at[t % 2]), w3[:, n * 128:(n + 1) * 128])
            hs.append((gate * jax.nn.sigmoid(gate) * up).astype(BF16))
        assert not ln_todo
        y = _dot(jnp.concatenate(hs, axis=1), w2[...])
        for j in range(NB):
            add_to_x(t, j, _block(y, j))

        @pl.when(layer == N_LAYERS - 1)
        def _():
            store_tile(t)
        return layer

    def run_layer(layer, carry):
        lax.fori_loop(0, NT, attention_tile, layer)

        @pl.when(layer == 0)
        def _():
            for c in ffn_copies:
                c.wait()
        lax.fori_loop(0, NT, ffn_tile, layer)
        return carry

    lax.fori_loop(0, N_LAYERS, run_layer, 0)
    for t in range(NT):
        o_copy(t).wait()


@jax.jit
def pallas_interleave_layers__sliding_local_dilated__glu_gated_swiglu__prompt_kernel(
    A_x: jax.Array,
    A_wqkv: jax.Array,
    A_wo: jax.Array,
    B_x: jax.Array,
    B_w1: jax.Array,
    B_w3: jax.Array,
    B_w2: jax.Array,
):
    del B_x
    anyspec = pl.BlockSpec(memory_space=pl.ANY)
    out = pl.pallas_call(
        _kernel,
        in_specs=[anyspec] * 6,
        out_specs=anyspec,
        out_shape=jax.ShapeDtypeStruct((S, D), A_x.dtype),
        scratch_shapes=[
            pltpu.VMEM((3, D, D), BF16),
            pltpu.VMEM((NB, D, 128), BF16),
            pltpu.VMEM((3, NB, D, 128), BF16),
            pltpu.VMEM((NB, D, 128), BF16),
            pltpu.VMEM((D, F), BF16),
            pltpu.VMEM((D, F), BF16),
            pltpu.VMEM((F, D), BF16),
            pltpu.VMEM((NT, TM, D), BF16),
            pltpu.VMEM((NT, NB, 8 * XP + G, 128), F32),
            pltpu.VMEM((2, NB, TM, 128), BF16),
            pltpu.VMEM((H * PITCH + DH, 128), U32),
            pltpu.VMEM((H * PITCH + DH, 128), U32),
            pltpu.VMEM((NB, TM, 128), F32),
            pltpu.VMEM((NB, HG * 8 + TM, 128), F32),
            pltpu.VMEM((NB, HG * 8 + TM, 128), F32),
            pltpu.VMEM((W + 1, TM, 128), F32),
            pltpu.VMEM((NB, TM, 128), BF16),
            pltpu.SemaphoreType.DMA((NT,)),
            pltpu.SemaphoreType.DMA((3 * NR + NB,)),
            pltpu.SemaphoreType.DMA((3,)),
            pltpu.SemaphoreType.DMA((NT,)),
        ],
        compiler_params=pltpu.CompilerParams(vmem_limit_bytes=100 * 1024 * 1024),
    )(A_x.reshape(S, D), A_wqkv, A_wo, B_w1, B_w3, B_w2)
    return out.reshape(1, S, D)
```

```python
import jax
import jax.numpy as jnp
from jax import lax
import jax.experimental.pallas as pl
import jax.experimental.pallas.tpu as pltpu

CFG = dict(LB0=2, LBS=2, DNB=2, GNB=2, KNB=1, QNB=1, ONB=2, ORD=1, R3=0)
S, D, F = 2048, 1024, 3584
H, DH, W, DIL = 32, 32, 8, 2
N_LAYERS = 2
TM = 256
NT = S // TM
G = TM // 8
HG = 16
NB = D // 128
HM, HD, HB = TM // 2, D // 2, NB // 2
XP = G + 1
PITCH = DH + 1
PR = 128
NR = D // 2 // PR
AHEAD = 3
F32, BF16, U32 = jnp.float32, jnp.bfloat16, jnp.uint32
SCALE = DH ** -0.5
LOG2E = 1.4426950408889634


def _dot(a, b):
    return jnp.dot(a, b, preferred_element_type=F32)


def _wide(ref, j0=0, j1=NB):
    return jnp.concatenate([ref[j] for j in range(j0, j1)], axis=1)


def _block(val, j):
    return val[:, j * 128:(j + 1) * 128]


def _lhs_terms(a11, a12, a21, a22):
    return [a11 + a22, a21 + a22, a11, a22, a11 + a12, a21 - a11, a12 - a22]


def _rhs_terms(b11, b12, b21, b22):
    return [b11 + b22, b11, b12 - b22, b21 - b11, b22, b11 + b12, b21 + b22]


def _rhs_sums(b11, b12, b21, b22):
    return [b11 + b22, b12 - b22, b21 - b11, b11 + b12, b21 + b22]


def _combine(m):
    m1, m2, m3, m4, m5, m6, m7 = m
    return (m1 + m4) + (m7 - m5), m3 + m5, m2 + m4, (m1 - m2) + (m3 + m6)


def _head_major_to_dim_major(val, buf):
    for h in range(H):
        buf[pl.ds(h * PITCH, DH), :] = val[h * DH:(h + 1) * DH]
    return jnp.concatenate([buf[pl.ds(d, H, stride=PITCH), :] for d in range(DH)], axis=0)


def _kernel(x_h, wqkv_h, wo_h, w1_h, w3_h, w2_h, o_h,
            wqkv_in, wo_in, wqkv, wo, w1, w3, w2, w1s, w3s, w2s, xio, xs, xl, hl, tbuf_a, tbuf_b,
            q_s, k_s, v_s, p_s, a_s, sem_x, sem_a, sem_w, sem_o):

    def x_copy(t):
        return pltpu.make_async_copy(x_h.at[pl.ds(t * TM, TM), :], xio.at[t], sem_x.at[t])

    def o_copy(t):
        return pltpu.make_async_copy(xio.at[t], o_h.at[pl.ds(t * TM, TM), :], sem_o.at[t])

    def qkv_copies(n):
        m = n // NR
        cols = pl.ds(pl.multiple_of(m * D, D), D)
        copies = []
        for r0 in (0, HD):
            rows = pl.ds(pl.multiple_of(r0 + (n % NR) * PR, PR), PR)
            copies.append(pltpu.make_async_copy(wqkv_h.at[rows, cols], wqkv_in.at[m, rows, :], sem_a.at[n]))
        return copies

    def wo_copies(j):
        return [pltpu.make_async_copy(wo_h.at[:, pl.ds(pl.multiple_of((j + j0) * 128, 128), 128)],
                                      wo_in.at[j + j0], sem_a.at[3 * NR + j]) for j0 in (0, HB)]

    ffn_copies = [pltpu.make_async_copy(src, dst, sem_w.at[n])
                  for n, (src, dst) in enumerate([(w1_h, w1), (w3_h, w3), (w2_h, w2)])]

    def x_rows(t, j, g0, ng):
        return jnp.concatenate([xs[t, j, pl.ds(g0 + g, 8, stride=XP), :] for g in range(ng)], axis=0)

    def add_to_x(t, j, y):
        for g in range(G):
            xs[t, j, pl.ds(g, 8, stride=XP), :] += y[g * 8:(g + 1) * 8]

    def load_tile(t):
        x_copy(t).wait()
        for j in range(NB):
            val = xio[t, :, j * 128:(j + 1) * 128].astype(F32)
            for s in range(8):
                xs[t, j, pl.ds(s * XP, G), :] = val[s * G:(s + 1) * G]

    def store_tile(t):
        for j in range(NB):
            val = jnp.concatenate([xs[t, j, pl.ds(s * XP, G), :] for s in range(8)], axis=0)
            xio[t, :, j * 128:(j + 1) * 128] = val.astype(BF16)
        o_copy(t).start()

    def normalized(t, g0, ng):
        xb = [x_rows(t, j, g0, ng) for j in range(NB)]
        tot = xb[0]
        for j in range(1, NB):
            tot = tot + xb[j]
        mean = jnp.sum(tot, axis=-1, keepdims=True) * (1.0 / D)
        cb = [b - mean for b in xb]
        sq = cb[0] * cb[0]
        for j in range(1, NB):
            sq = sq + cb[j] * cb[j]
        rstd = lax.rsqrt(jnp.sum(sq, axis=-1, keepdims=True) * (1.0 / D) + 1e-5)
        return [c * rstd for c in cb]

    def layernorm(t, slot, g0):
        top, bot = normalized(t, g0, 2), normalized(t, g0 + G // 2, 2)
        r0 = g0 * 8 if isinstance(g0, int) else pl.multiple_of(g0 * 8, 16)
        for j in range(NB // 2):
            terms = _lhs_terms(top[j], top[j + NB // 2], bot[j], bot[j + NB // 2])
            for i in range(7):
                xl[slot, i, j, pl.ds(r0, 16), :] = terms[i].astype(BF16)

    def next_tile_layernorm(t):
        nt = (t + 1) % NT
        todo = list(range(0, G // 2, 2))

        def step(n):
            for _ in range(min(n, len(todo))):
                layernorm(nt, nt % 2, todo.pop(0))
        return step, todo

    n_steps = 3 * NR
    n_a = n_steps - HB

    def prefetch(n):
        @pl.when(n < n_steps)
        def _():
            for c in qkv_copies(n):
                c.start()

        @pl.when(jnp.logical_and(n >= n_a, n < n_steps))
        def _():
            for c in wo_copies(n - n_a):
                c.start()

    def reorder_qkv_columns(n):
        for c in qkv_copies(n):
            c.wait()
        m = n // NR
        r = pl.multiple_of((n % NR) * PR, PR)
        val = jnp.concatenate([wqkv_in[m, pl.ds(r0 + r, PR), :] for r0 in (0, HD)], axis=0)
        t = pltpu.bitcast(val, U32).T
        val = pltpu.bitcast(_head_major_to_dim_major(t, tbuf_a).T, BF16).astype(F32)
        for j in range(HB):
            terms = _rhs_terms(_block(val[:PR], j), _block(val[:PR], j + HB),
                               _block(val[PR:], j), _block(val[PR:], j + HB))
            for i in range(7):
                wqkv[m, i, j, pl.ds(r, PR), :] = terms[i].astype(BF16)

    def prologue_a(n, carry):
        prefetch(n + AHEAD)
        reorder_qkv_columns(n)
        layernorm(0, 0, 2 * n)
        k_s[n, pl.ds(TM, HG * 8), :] = jnp.zeros((HG * 8, 128), F32)
        v_s[n, pl.ds(TM, HG * 8), :] = jnp.zeros((HG * 8, 128), F32)
        return carry

    def prologue_b(n, carry):
        prefetch(n + AHEAD)
        j = n - n_a
        for c in wo_copies(j):
            c.wait()
        reorder_qkv_columns(n)
        left, right = [
            pltpu.bitcast(_head_major_to_dim_major(pltpu.bitcast(wo_in[j + j0].astype(F32), U32), tbuf_b), F32)
            for j0 in (0, HB)]
        terms = _rhs_terms(left[:HD], right[:HD], left[HD:], right[HD:])
        for i in range(7):
            wo[i, j] = terms[i].astype(BF16)
        return carry

    assert n_a == NB and 2 * n_a * 2 == G
    x_copy(0).start()
    for n in range(AHEAD):
        for c in qkv_copies(n):
            c.start()
    load_tile(0)
    lax.fori_loop(0, n_a, prologue_a, 0)
    lax.fori_loop(n_a, n_steps, prologue_b, 0)
    for t in range(1, NT):
        x_copy(t).start()
    for c in ffn_copies:
        c.start()

    def project(t, m, j0, j1):
        c11, c12, c21, c22 = _combine([_dot(_wide(xl.at[t % 2, i], 0, HB), _wide(wqkv.at[m, i], j0, j1))
                                       for i in range(7)])
        for j in range(j0, j1):
            yield j, jnp.concatenate([_block(c11, j - j0), _block(c21, j - j0)], axis=0)
            yield j + HB, jnp.concatenate([_block(c12, j - j0), _block(c22, j - j0)], axis=0)

    def project_with_halo(t, dst, m, j0, j1):
        sub = lax.broadcasted_iota(jnp.int32, (HG * 8, 128), 0) % 8
        for j, new in project(t, m, j0, j1):
            old = dst[j, pl.ds(TM, HG * 8), :]
            prev = jnp.where(t == 0, jnp.broadcast_to(new[0:1, :], (HG * 8, 128)),
                             pltpu.roll(old, HG * 8 - 7, 0))
            dst[j, pl.ds(0, HG * 8), :] = jnp.where(sub == 0, prev, pltpu.roll(new[TM - HG * 8:, :], 1, 0))
            dst[j, pl.ds(HG * 8, TM), :] = new

    def softmax_weights(t, g):
        r = g * 8
        qs = [q_s[j, r:r + 8, :] for j in range(NB)]
        logits = []
        for w in range(W):
            rk = r + (HG - DIL * w) * 8
            a = qs[0] * k_s[0, rk:rk + 8, :]
            for j in range(1, NB):
                a = a + qs[j] * k_s[j, rk:rk + 8, :]
            if CFG['R3']:
                a = (a + pltpu.roll(a, 64, 1)) + (pltpu.roll(a, 32, 1) + pltpu.roll(a, 96, 1))
            else:
                a = a + pltpu.roll(a, 64, 1)
                a = a + pltpu.roll(a, 32, 1)
            if g < DIL * w:
                pos = t * TM + g + G * lax.broadcasted_iota(jnp.int32, (8, 128), 0)
                a = jnp.where(pos >= DIL * w, a, -1e9 / SCALE)
            logits.append(a)
        mx = logits[0]
        for w in range(1, W):
            mx = jnp.maximum(mx, logits[w])
        ps = [jnp.exp2((a - mx) * (SCALE * LOG2E)) for a in logits]
        den = ps[0]
        for w in range(1, W):
            den = den + ps[w]
        for w in range(W):
            p_s[w, r:r + 8, :] = ps[w]
        p_s[W, r:r + 8, :] = 1.0 / den

    def weighted_values(j):
        def rows(jj, r):
            a = p_s[0, r:r + 16, :] * v_s[jj, r + HG * 8:r + HG * 8 + 16, :]
            for w in range(1, W):
                rk = r + (HG - DIL * w) * 8
                a = a + p_s[w, r:r + 16, :] * v_s[jj, rk:rk + 16, :]
            return a * p_s[W, r:r + 16, :]
        for r in range(0, HM, 16):
            terms = _lhs_terms(rows(j, r), rows(j + HB, r), rows(j, r + HM), rows(j + HB, r + HM))
            for i in range(7):
                a_s[i, j, r:r + 16, :] = terms[i].astype(BF16)

    def add_quadrants_to_x(t, j0, y):
        for e in range(y[0].shape[1] // 128):
            add_to_x(t, j0 + e, jnp.concatenate([_block(y[0], e), _block(y[2], e)], axis=0))
            add_to_x(t, HB + j0 + e, jnp.concatenate([_block(y[1], e), _block(y[3], e)], axis=0))

    def attention_tile(t, layer):
        @pl.when(jnp.logical_and(layer == 0, t + 1 < NT))
        def _():
            load_tile(t + 1)

        ln_step, ln_todo = next_tile_layernorm(t)
        knb, qnb, onb = CFG['KNB'], CFG['QNB'], CFG['ONB']
        ks = [(0, j) for j in range(0, HB, knb)]
        qs = [(1, j) for j in range(0, HB, qnb)]
        order = ks + qs if CFG['ORD'] == 0 else [e for pr in zip(ks, qs) for e in pr]
        for is_q, j in order:
            if is_q:
                for jj, val in project(t, 0, j, j + qnb):
                    q_s[jj] = val
            else:
                project_with_halo(t, k_s, 1, j, j + knb)
            ln_step(CFG.get('LA', -(-8 // len(order))))
        assert not ln_todo
        for c in range(2):
            project_with_halo(t, v_s, 2, 2 * c, 2 * c + 2)
            for g in range(c * G // 2, (c + 1) * G // 2):
                softmax_weights(t, g)
        for j in range(2):
            weighted_values(j)
        for c in range(2):
            for n in range(0, HB, onb):
                y = _combine([_dot(_wide(a_s.at[i], 2 * c, 2 * c + 2),
                                   _wide(wo.at[i, :, c * 256:(c + 1) * 256, :], n, n + onb)) for i in range(7)])
                add_quadrants_to_x(t, n, y)
                if c == 0:
                    for j in range(2 + 2 * n // HB, 2 + 2 * (n + onb) // HB):
                        weighted_values(j)
        return layer

    def ffn_tile(t, layer):
        ln_step, ln_todo = next_tile_layernorm(t)
        slot = t % 2
        hd, hf, nf = D // 2, F // 2, F // 256

        def rhs(w, ws, i, n, nb, hk, hn):
            if i == 1:
                return w[0:hk, n * 128:(n + nb) * 128]
            if i == 4:
                return w[hk:2 * hk, hn + n * 128:hn + (n + nb) * 128]
            return _wide(ws.at[{0: 0, 2: 1, 3: 2, 5: 3, 6: 4}[i]], n, n + nb)

        gnb, dnb = CFG['GNB'], CFG['DNB']
        for n in range(0, nf, gnb):
            gate = _combine([_dot(_wide(xl.at[slot, i], 0, NB // 2), rhs(w1, w1s, i, n, gnb, hd, hf)) for i in range(7)])
            if n >= CFG['LB0']:
                ln_step(CFG['LBS'])
            up = _combine([_dot(_wide(xl.at[slot, i], 0, NB // 2), rhs(w3, w3s, i, n, gnb, hd, hf)) for i in range(7)])
            terms = _lhs_terms(*[g * jax.nn.sigmoid(g) * u for g, u in zip(gate, up)])
            for i in range(7):
                for e in range(gnb):
                    hl[i, n + e] = _block(terms[i], e).astype(BF16)
        assert not ln_todo
        for n in range(0, NB // 2, dnb):
            y = _combine([_dot(_wide(hl.at[i], 0, nf), rhs(w2, w2s, i, n, dnb, hf, hd)) for i in range(7)])
            add_quadrants_to_x(t, n, y)

        @pl.when(layer == N_LAYERS - 1)
        def _():
            store_tile(t)
        return layer

    def run_layer(layer, carry):
        lax.fori_loop(0, NT, attention_tile, layer)

        @pl.when(layer == 0)
        def _():
            for c in ffn_copies:
                c.wait()
            for w, ws in ((w1, w1s), (w3, w3s), (w2, w2s)):
                hk, hn = w.shape[0] // 2, w.shape[1] // 2

                def weight_sums(i, carry, w=w, ws=ws, hk=hk, hn=hn):
                    r = pl.multiple_of(i * 32, 32)
                    for n in range(hn // 128):
                        quads = [w[pl.ds(r0 + r, 32), c0 + n * 128:c0 + (n + 1) * 128].astype(F32)
                                 for r0 in (0, hk) for c0 in (0, hn)]
                        for k, val in enumerate(_rhs_sums(*quads)):
                            ws[k, n, pl.ds(r, 32), :] = val.astype(BF16)
                    return carry
                lax.fori_loop(0, hk // 32, weight_sums, 0)
        lax.fori_loop(0, NT, ffn_tile, layer)
        return carry

    lax.fori_loop(0, N_LAYERS, run_layer, 0)
    for t in range(NT):
        o_copy(t).wait()


@jax.jit
def pallas_interleave_layers__sliding_local_dilated__glu_gated_swiglu__prompt_kernel(
    A_x: jax.Array,
    A_wqkv: jax.Array,
    A_wo: jax.Array,
    B_x: jax.Array,
    B_w1: jax.Array,
    B_w3: jax.Array,
    B_w2: jax.Array,
):
    del B_x
    anyspec = pl.BlockSpec(memory_space=pl.ANY)
    out = pl.pallas_call(
        _kernel,
        in_specs=[anyspec] * 6,
        out_specs=anyspec,
        out_shape=jax.ShapeDtypeStruct((S, D), A_x.dtype),
        scratch_shapes=[
            pltpu.VMEM((3, D, D), BF16),
            pltpu.VMEM((NB, D, 128), BF16),
            pltpu.VMEM((3, 7, HB, HD, 128), BF16),
            pltpu.VMEM((7, HB, HD, 128), BF16),
            pltpu.VMEM((D, F), BF16),
            pltpu.VMEM((D, F), BF16),
            pltpu.VMEM((F, D), BF16),
            pltpu.VMEM((5, F // 256, D // 2, 128), BF16),
            pltpu.VMEM((5, F // 256, D // 2, 128), BF16),
            pltpu.VMEM((5, NB // 2, F // 2, 128), BF16),
            pltpu.VMEM((NT, TM, D), BF16),
            pltpu.VMEM((NT, NB, 8 * XP + G, 128), F32),
            pltpu.VMEM((2, 7, NB // 2, TM // 2, 128), BF16),
            pltpu.VMEM((7, F // 256, TM // 2, 128), BF16),
            pltpu.VMEM((H * PITCH + DH, 128), U32),
            pltpu.VMEM((H * PITCH + DH, 128), U32),
            pltpu.VMEM((NB, TM, 128), F32),
            pltpu.VMEM((NB, HG * 8 + TM, 128), F32),
            pltpu.VMEM((NB, HG * 8 + TM, 128), F32),
            pltpu.VMEM((W + 1, TM, 128), F32),
            pltpu.VMEM((7, HB, HM, 128), BF16),
            pltpu.SemaphoreType.DMA((NT,)),
            pltpu.SemaphoreType.DMA((3 * NR + HB,)),
            pltpu.SemaphoreType.DMA((3,)),
            pltpu.SemaphoreType.DMA((NT,)),
        ],
        compiler_params=pltpu.CompilerParams(vmem_limit_bytes=116 * 1024 * 1024),
    )(A_x.reshape(S, D), A_wqkv, A_wo, B_w1, B_w3, B_w2)
    return out.reshape(1, S, D)
```

```python
import jax
import jax.numpy as jnp
from jax import lax
import jax.experimental.pallas as pl
import jax.experimental.pallas.tpu as pltpu

CFG = dict(LB0=2, LBS=2, DNB=2, GNB=2, KNB=2, QNB=2, ONB=4, ORD=1, R3=1, PLAIN=(), QH=0, WK=2, VNB=1, SM=1, QU=0, OU=0, WU=0, HU=0, XU=1, W2U=0, LATE=1)
S, D, F = 2048, 1024, 3584
H, DH, W, DIL = 32, 32, 8, 2
N_LAYERS = 2
TM = 256
NT = S // TM
G = TM // 8
HG = 16
NB = D // 128
HM, HD, HB = TM // 2, D // 2, NB // 2
XP = G + 1
PITCH = DH + 1
PR = 128
NR = D // 2 // PR
AHEAD = 3
F32, BF16, U32 = jnp.float32, jnp.bfloat16, jnp.uint32
SCALE = DH ** -0.5
LOG2E = 1.4426950408889634


def _dot(a, b):
    return jnp.dot(a, b, preferred_element_type=F32)


def _wide(ref, j0=0, j1=NB):
    return jnp.concatenate([pltpu.bitcast(ref[j], BF16) if ref.dtype == U32 else ref[j] for j in range(j0, j1)], axis=1)


def _pack(val):
    return pltpu.bitcast(val.astype(BF16), U32)


def _block(val, j):
    return val[:, j * 128:(j + 1) * 128]


def _lhs_terms(a11, a12, a21, a22):
    return [a11 + a22, a21 + a22, a11, a22, a11 + a12, a21 - a11, a12 - a22]


def _rhs_terms(b11, b12, b21, b22):
    return [b11 + b22, b11, b12 - b22, b21 - b11, b22, b11 + b12, b21 + b22]


def _rhs_sums(b11, b12, b21, b22):
    return [b11 + b22, b12 - b22, b21 - b11, b11 + b12, b21 + b22]


def _strassen(product):
    m2 = product(1)
    m4 = product(3)
    c21 = m2 + m4
    m3 = product(2)
    c22 = m3 - m2
    m5 = product(4)
    c12 = m3 + m5
    c11 = m4 - m5
    m1 = product(0)
    c22 = (c22 + m1) + product(5)
    c11 = (c11 + m1) + product(6)
    return c11, c12, c21, c22


def _head_major_to_dim_major(val, buf):
    for h in range(H):
        buf[pl.ds(h * PITCH, DH), :] = val[h * DH:(h + 1) * DH]
    return jnp.concatenate([buf[pl.ds(d, H, stride=PITCH), :] for d in range(DH)], axis=0)


def _kernel(x_h, wqkv_h, wo_h, w1_h, w3_h, w2_h, o_h,
            wqkv_in, wo_in, wqkv, wo, w1, w3, w2, w1s, w3s, w2s, xio, xs, xl, hl, tbuf_a, tbuf_b,
            q_s, k_s, v_s, p_s, a_s, sem_x, sem_a, sem_w, sem_o):

    def x_copy(t):
        return pltpu.make_async_copy(x_h.at[pl.ds(t * TM, TM), :], xio.at[t], sem_x.at[t])

    def o_copy(t):
        return pltpu.make_async_copy(xio.at[t], o_h.at[pl.ds(t * TM, TM), :], sem_o.at[t])

    def qkv_copies(n):
        m = n // NR
        cols = pl.ds(pl.multiple_of(m * D, D), D)
        copies = []
        for r0 in (0, HD):
            rows = pl.ds(pl.multiple_of(r0 + (n % NR) * PR, PR), PR)
            copies.append(pltpu.make_async_copy(wqkv_h.at[rows, cols], wqkv_in.at[m, rows, :], sem_a.at[n]))
        return copies

    def wo_copies(j):
        return [pltpu.make_async_copy(wo_h.at[:, pl.ds(pl.multiple_of((j + j0) * 128, 128), 128)],
                                      wo_in.at[j + j0], sem_a.at[3 * NR + j]) for j0 in (0, HB)]

    ffn_copies = [pltpu.make_async_copy(src, dst, sem_w.at[n])
                  for n, (src, dst) in enumerate([(w1_h, w1), (w3_h, w3), (w2_h, w2)])]

    def x_rows(t, j, g0, ng):
        return jnp.concatenate([xs[t, j, pl.ds(g0 + g, 8, stride=XP), :] for g in range(ng)], axis=0)

    def add_to_x(t, j, y):
        for g in range(G):
            xs[t, j, pl.ds(g, 8, stride=XP), :] += y[g * 8:(g + 1) * 8]

    def load_tile(t):
        x_copy(t).wait()
        for j in range(NB):
            val = xio[t, :, j * 128:(j + 1) * 128].astype(F32)
            for s in range(8):
                xs[t, j, pl.ds(s * XP, G), :] = val[s * G:(s + 1) * G]

    def store_tile(t):
        for j in range(NB):
            val = jnp.concatenate([xs[t, j, pl.ds(s * XP, G), :] for s in range(8)], axis=0)
            xio[t, :, j * 128:(j + 1) * 128] = val.astype(BF16)
        o_copy(t).start()

    def normalized(t, g0, ng):
        xb = [x_rows(t, j, g0, ng) for j in range(NB)]
        tot = xb[0]
        for j in range(1, NB):
            tot = tot + xb[j]
        mean = jnp.sum(tot, axis=-1, keepdims=True) * (1.0 / D)
        cb = [b - mean for b in xb]
        sq = cb[0] * cb[0]
        for j in range(1, NB):
            sq = sq + cb[j] * cb[j]
        rstd = lax.rsqrt(jnp.sum(sq, axis=-1, keepdims=True) * (1.0 / D) + 1e-5)
        return [c * rstd for c in cb]

    def layernorm(t, slot, g0):
        top, bot = normalized(t, g0, 2), normalized(t, g0 + G // 2, 2)
        r0 = g0 * 4 if isinstance(g0, int) else pl.multiple_of(g0 * 4, 8)
        for j in range(NB // 2):
            terms = _lhs_terms(top[j], top[j + HB], bot[j], bot[j + HB])
            if CFG['PLAIN']:
                terms += [top[j + HB], bot[j]]
            for i in range(len(terms)):
                if CFG['XU']:
                    xl[slot, i, j, pl.ds(r0, 8), :] = _pack(terms[i])
                else:
                    xl[slot, i, j, pl.ds(2 * r0 if isinstance(r0, int) else pl.multiple_of(2 * r0, 16), 16), :] = terms[i].astype(BF16)

    def next_tile_layernorm(t):
        nt = (t + 1) % NT
        todo = list(range(0, G // 2, 2))

        def step(n):
            for _ in range(min(n, len(todo))):
                layernorm(nt, nt % 2, todo.pop(0))
        return step, todo

    n_steps = 3 * NR
    n_a = n_steps - HB

    def prefetch(n):
        @pl.when(n < n_steps)
        def _():
            for c in qkv_copies(n):
                c.start()

        @pl.when(jnp.logical_and(n >= n_a, n < n_steps))
        def _():
            for c in wo_copies(n - n_a):
                c.start()

    def reorder_qkv_columns(n):
        for c in qkv_copies(n):
            c.wait()
        m = n // NR
        r = pl.multiple_of((n % NR) * PR, PR)
        val = jnp.concatenate([wqkv_in[m, pl.ds(r0 + r, PR), :] for r0 in (0, HD)], axis=0)
        t = pltpu.bitcast(val, U32).T
        val = pltpu.bitcast(_head_major_to_dim_major(t, tbuf_a).T, BF16).astype(F32)
        for j in range(HB):
            terms = _rhs_terms(_block(val[:PR], j), _block(val[:PR], j + HB),
                               _block(val[PR:], j), _block(val[PR:], j + HB))
            for i in range(7):
                if CFG['QU']:
                    wqkv[m, i, j, pl.ds(pl.multiple_of(r // 2, PR // 2), PR // 2), :] = _pack(terms[i])
                else:
                    wqkv[m, i, j, pl.ds(r, PR), :] = terms[i].astype(BF16)

    def prologue_a(n, carry):
        prefetch(n + AHEAD)
        reorder_qkv_columns(n)
        layernorm(0, 0, 2 * n)
        k_s[n, pl.ds(TM, HG * 8), :] = jnp.zeros((HG * 8, 128), F32)
        v_s[n, pl.ds(TM, HG * 8), :] = jnp.zeros((HG * 8, 128), F32)
        return carry

    def prologue_b(n, carry):
        prefetch(n + AHEAD)
        j = n - n_a
        for c in wo_copies(j):
            c.wait()
        reorder_qkv_columns(n)
        left, right = [
            pltpu.bitcast(_head_major_to_dim_major(pltpu.bitcast(wo_in[j + j0].astype(F32), U32), tbuf_b), F32)
            for j0 in (0, HB)]
        terms = _rhs_terms(left[:HD], right[:HD], left[HD:], right[HD:])
        for i in range(7):
            wo[i, j] = _pack(terms[i]) if CFG['OU'] else terms[i].astype(BF16)
        return carry

    assert n_a == NB and 2 * n_a * 2 == G
    x_copy(0).start()
    for n in range(AHEAD):
        for c in qkv_copies(n):
            c.start()
    load_tile(0)
    lax.fori_loop(0, n_a, prologue_a, 0)
    lax.fori_loop(n_a, n_steps, prologue_b, 0)
    for t in range(1, NT):
        x_copy(t).start()
    for c in ffn_copies:
        c.start()

    def project(t, m, j0, j1):
        if m in CFG['PLAIN']:
            lhs = jnp.concatenate([jnp.concatenate([_wide(xl.at[t % 2, i], 0, HB) for i in pr], axis=1)
                                   for pr in ((2, 7), (8, 3))], axis=0)
            rhs = jnp.concatenate([jnp.concatenate([_wide(wqkv.at[m, i], j0, j1) for i in pr], axis=1)
                                   for pr in ((1, 7), (8, 4))], axis=0)
            if m == 0 and CFG['QH']:
                val = jnp.concatenate([_dot(lhs[:HM], rhs), _dot(lhs[HM:], rhs)], axis=0)
            else:
                val = _dot(lhs, rhs)
            for j in range(j0, j1):
                yield j, _block(val, j - j0)
                yield j + HB, _block(val, j - j0 + j1 - j0)
            return
        c11, c12, c21, c22 = _strassen(lambda i: _dot(_wide(xl.at[t % 2, i], 0, HB), _wide(wqkv.at[m, i], j0, j1)))
        for j in range(j0, j1):
            yield j, jnp.concatenate([_block(c11, j - j0), _block(c21, j - j0)], axis=0)
            yield j + HB, jnp.concatenate([_block(c12, j - j0), _block(c22, j - j0)], axis=0)

    def project_with_halo(t, dst, m, j0, j1):
        sub = lax.broadcasted_iota(jnp.int32, (HG * 8, 128), 0) % 8
        for j, new in project(t, m, j0, j1):
            old = dst[j, pl.ds(TM, HG * 8), :]
            prev = jnp.where(t == 0, jnp.broadcast_to(new[0:1, :], (HG * 8, 128)),
                             pltpu.roll(old, HG * 8 - 7, 0))
            dst[j, pl.ds(0, HG * 8), :] = jnp.where(sub == 0, prev, pltpu.roll(new[TM - HG * 8:, :], 1, 0))
            dst[j, pl.ds(HG * 8, TM), :] = new

    def softmax_weights(t, g):
        r = g * 8
        qs = [q_s[j, r:r + 8, :] for j in range(NB)]
        logits = []
        for w in range(W):
            rk = r + (HG - DIL * w) * 8
            a = qs[0] * k_s[0, rk:rk + 8, :]
            for j in range(1, NB):
                a = a + qs[j] * k_s[j, rk:rk + 8, :]
            if CFG['R3']:
                a = (a + pltpu.roll(a, 64, 1)) + (pltpu.roll(a, 32, 1) + pltpu.roll(a, 96, 1))
            else:
                a = a + pltpu.roll(a, 64, 1)
                a = a + pltpu.roll(a, 32, 1)
            if g < DIL * w:
                pos = t * TM + g + G * lax.broadcasted_iota(jnp.int32, (8, 128), 0)
                a = jnp.where(pos >= DIL * w, a, -1e9 / SCALE)
            logits.append(a)
        mx = logits[0]
        for w in range(1, W):
            mx = jnp.maximum(mx, logits[w])
        ps = [jnp.exp2((a - mx) * (SCALE * LOG2E)) for a in logits]
        den = ps[0]
        for w in range(1, W):
            den = den + ps[w]
        inv = 1.0 / den
        for w in range(W):
            p_s[w, r:r + 8, :] = ps[w] if CFG['LATE'] else ps[w] * inv
        if CFG['LATE']:
            p_s[W, r:r + 8, :] = inv

    def weighted_values(j):
        def rows(jj, r):
            a = p_s[0, r:r + 16, :] * v_s[jj, r + HG * 8:r + HG * 8 + 16, :]
            for w in range(1, W):
                rk = r + (HG - DIL * w) * 8
                a = a + p_s[w, r:r + 16, :] * v_s[jj, rk:rk + 16, :]
            return a * p_s[W, r:r + 16, :] if CFG['LATE'] else a
        for r in range(0, HM, 16):
            terms = _lhs_terms(rows(j, r), rows(j + HB, r), rows(j, r + HM), rows(j + HB, r + HM))
            for i in range(7):
                a_s[i, j, r // 2:r // 2 + 8, :] = _pack(terms[i])

    def add_quadrants_to_x(t, j0, y):
        for e in range(y[0].shape[1] // 128):
            add_to_x(t, j0 + e, jnp.concatenate([_block(y[0], e), _block(y[2], e)], axis=0))
            add_to_x(t, HB + j0 + e, jnp.concatenate([_block(y[1], e), _block(y[3], e)], axis=0))

    def attention_tile(t, layer):
        @pl.when(jnp.logical_and(layer == 0, t + 1 < NT))
        def _():
            load_tile(t + 1)

        ln_step, ln_todo = next_tile_layernorm(t)
        knb, qnb, onb = CFG['KNB'], CFG['QNB'], CFG['ONB']
        ks = [(0, j) for j in range(0, HB, knb)]
        qs = [(1, j) for j in range(0, HB, qnb)]
        order = [ks + qs, [e for pr in zip(ks, qs) for e in pr], [e for pr in zip(qs, ks) for e in pr], qs + ks][CFG['ORD']]
        for is_q, j in order:
            if is_q:
                for jj, val in project(t, 0, j, j + qnb):
                    q_s[jj] = val
            else:
                project_with_halo(t, k_s, 1, j, j + knb)
            ln_step(CFG.get('LA', -(-8 // len(order))))
        assert not ln_todo
        vnb, wk = CFG['VNB'], CFG['WK']
        kb = HB // wk
        orow = 64 if CFG['OU'] else 128
        if CFG['SM'] == 0:
            for g in range(G):
                softmax_weights(t, g)
        for j in range(0, HB, vnb):
            project_with_halo(t, v_s, 2, j, j + vnb)
            if CFG['SM'] == 1:
                for g in range(j * G // HB, (j + vnb) * G // HB):
                    softmax_weights(t, g)
            if CFG['SM'] == 2 and j == 0:
                for g in range(G):
                    softmax_weights(t, g)
            if CFG['SM'] == 3 and j == 0:
                for g in range(G // 2):
                    softmax_weights(t, g)
                    softmax_weights(t, g + G // 2)
        for j in range(kb):
            weighted_values(j)
        for c in range(wk):
            for n in range(0, HB, onb):
                y = _strassen(lambda i: _dot(_wide(a_s.at[i], c * kb, (c + 1) * kb),
                                   _wide(wo.at[i, :, c * kb * orow:(c + 1) * kb * orow, :], n, n + onb)))
                add_quadrants_to_x(t, n, y)
                if c + 1 < wk:
                    for j in range((c + 1) * kb + kb * n // HB, (c + 1) * kb + kb * (n + onb) // HB):
                        weighted_values(j)
        return layer

    def ffn_tile(t, layer):
        ln_step, ln_todo = next_tile_layernorm(t)
        slot = t % 2
        hd, hf, nf = D // 2, F // 2, F // 256

        def rhs(w, ws, i, n, nb, hk, hn):
            if i == 1:
                return w[0:hk, n * 128:(n + nb) * 128]
            if i == 4:
                return w[hk:2 * hk, hn + n * 128:hn + (n + nb) * 128]
            return _wide(ws.at[{0: 0, 2: 1, 3: 2, 5: 3, 6: 4}[i]], n, n + nb)

        gnb, dnb = CFG['GNB'], CFG['DNB']
        for n in range(0, nf, gnb):
            gate = _strassen(lambda i: _dot(_wide(xl.at[slot, i], 0, NB // 2), rhs(w1, w1s, i, n, gnb, hd, hf)))
            if n >= CFG['LB0']:
                ln_step(CFG['LBS'])
            up = _strassen(lambda i: _dot(_wide(xl.at[slot, i], 0, NB // 2), rhs(w3, w3s, i, n, gnb, hd, hf)))
            terms = _lhs_terms(*[g * jax.nn.sigmoid(g) * u for g, u in zip(gate, up)])
            for i in range(7):
                for e in range(gnb):
                    hl[i, n + e] = _pack(_block(terms[i], e)) if CFG['HU'] else _block(terms[i], e).astype(BF16)
        assert not ln_todo
        for n in range(0, NB // 2, dnb):
            y = _strassen(lambda i: _dot(_wide(hl.at[i], 0, nf), rhs(w2, w2s, i, n, dnb, hf, hd)))
            add_quadrants_to_x(t, n, y)

        @pl.when(layer == N_LAYERS - 1)
        def _():
            store_tile(t)
        return layer

    def run_layer(layer, carry):
        lax.fori_loop(0, NT * CFG.get('AR', 1), lambda t, c: attention_tile(t % NT, c + t // NT) * 0 + c, layer)

        @pl.when(layer == 0)
        def _():
            for c in ffn_copies:
                c.wait()
            for w, ws in ((w1, w1s), (w3, w3s), (w2, w2s)):
                hk, hn = w.shape[0] // 2, w.shape[1] // 2

                def weight_sums(i, carry, w=w, ws=ws, hk=hk, hn=hn):
                    r = pl.multiple_of(i * 32, 32)
                    for n in range(hn // 128):
                        quads = [w[pl.ds(r0 + r, 32), c0 + n * 128:c0 + (n + 1) * 128].astype(F32)
                                 for r0 in (0, hk) for c0 in (0, hn)]
                        for k, val in enumerate(_rhs_sums(*quads)):
                            if ws.dtype == U32:
                                ws[k, n, pl.ds(pl.multiple_of(i * 16, 16), 16), :] = _pack(val)
                            else:
                                ws[k, n, pl.ds(r, 32), :] = val.astype(BF16)
                    return carry
                lax.fori_loop(0, hk // 32, weight_sums, 0)
        lax.fori_loop(0, NT, ffn_tile, layer)
        return carry

    lax.fori_loop(0, N_LAYERS, run_layer, 0)
    for t in range(NT):
        o_copy(t).wait()


@jax.jit
def pallas_interleave_layers__sliding_local_dilated__glu_gated_swiglu__prompt_kernel(
    A_x: jax.Array,
    A_wqkv: jax.Array,
    A_wo: jax.Array,
    B_x: jax.Array,
    B_w1: jax.Array,
    B_w3: jax.Array,
    B_w2: jax.Array,
):
    del B_x
    anyspec = pl.BlockSpec(memory_space=pl.ANY)
    out = pl.pallas_call(
        _kernel,
        in_specs=[anyspec] * 6,
        out_specs=anyspec,
        out_shape=jax.ShapeDtypeStruct((S, D), A_x.dtype),
        scratch_shapes=[
            pltpu.VMEM((3, D, D), BF16),
            pltpu.VMEM((NB, D, 128), BF16),
            pltpu.VMEM((3, 7, HB, HD // 2, 128), U32) if CFG['QU'] else pltpu.VMEM((3, 7, HB, HD, 128), BF16),
            pltpu.VMEM((7, HB, HD // 2, 128), U32) if CFG['OU'] else pltpu.VMEM((7, HB, HD, 128), BF16),
            pltpu.VMEM((D, F), BF16),
            pltpu.VMEM((D, F), BF16),
            pltpu.VMEM((F, D), BF16),
            pltpu.VMEM((5, F // 256, HD // 2, 128), U32) if CFG['WU'] else pltpu.VMEM((5, F // 256, HD, 128), BF16),
            pltpu.VMEM((5, F // 256, HD // 2, 128), U32) if CFG['WU'] else pltpu.VMEM((5, F // 256, HD, 128), BF16),
            pltpu.VMEM((5, HB, F // 4, 128), U32) if CFG['W2U'] else pltpu.VMEM((5, HB, F // 2, 128), BF16),
            pltpu.VMEM((NT, TM, D), BF16),
            pltpu.VMEM((NT, NB, 8 * XP + G, 128), F32),
            pltpu.VMEM((2, 7, HB, HM // 2, 128), U32) if CFG['XU'] else pltpu.VMEM((2, 7, HB, HM, 128), BF16),
            pltpu.VMEM((7, F // 256, HM // 2, 128), U32) if CFG['HU'] else pltpu.VMEM((7, F // 256, HM, 128), BF16),
            pltpu.VMEM((H * PITCH + DH, 128), U32),
            pltpu.VMEM((H * PITCH + DH, 128), U32),
            pltpu.VMEM((NB, TM, 128), F32),
            pltpu.VMEM((NB, HG * 8 + TM, 128), F32),
            pltpu.VMEM((NB, HG * 8 + TM, 128), F32),
            pltpu.VMEM((W + 1, TM, 128), F32),
            pltpu.VMEM((7, HB, HM // 2, 128), U32),
            pltpu.SemaphoreType.DMA((NT,)),
            pltpu.SemaphoreType.DMA((3 * NR + HB,)),
            pltpu.SemaphoreType.DMA((3,)),
            pltpu.SemaphoreType.DMA((NT,)),
        ],
        compiler_params=pltpu.CompilerParams(vmem_limit_bytes=116 * 1024 * 1024),
    )(A_x.reshape(S, D), A_wqkv, A_wo, B_w1, B_w3, B_w2)
    return out.reshape(1, S, D)
```

```python
import jax
import jax.numpy as jnp
from jax import lax
import jax.experimental.pallas as pl
import jax.experimental.pallas.tpu as pltpu

S, D, F = 2048, 1024, 3584
H, DH, W, DIL = 32, 32, 8, 2
N_LAYERS = 2
TM = 256
NT = S // TM
G = TM // 8
HG = 16
NB = D // 128
HM, HD, HB = TM // 2, D // 2, NB // 2
HF, FB = F // 2, F // 256
XP = G + 1
PITCH = DH + 1
PR = 128
NR = D // 2 // PR
AHEAD = 4
F32, BF16, U32 = jnp.float32, jnp.bfloat16, jnp.uint32
SCALE = DH ** -0.5
LOG2E = 1.4426950408889634


def _dot(a, b):
    return jnp.dot(a, b, preferred_element_type=F32)


def _wide(ref, j0, j1):
    blocks = [ref[j] for j in range(j0, j1)]
    if ref.dtype == U32:
        blocks = [pltpu.bitcast(b, BF16) for b in blocks]
    return jnp.concatenate(blocks, axis=1)


def _pack(val):
    return pltpu.bitcast(val.astype(BF16), U32)


def _block(val, j):
    return val[:, j * 128:(j + 1) * 128]


def _lhs_terms(a11, a12, a21, a22):
    return [a11 + a22, a21 + a22, a11, a22, a11 + a12, a21 - a11, a12 - a22]


def _rhs_terms(b11, b12, b21, b22):
    return [b11 + b22, b11, b12 - b22, b21 - b11, b22, b11 + b12, b21 + b22]


RHS_SUMS = (0, 2, 3, 5, 6)


def _strassen(product):
    m2 = product(1)
    m4 = product(3)
    c21 = m2 + m4
    m3 = product(2)
    c22 = m3 - m2
    m5 = product(4)
    c12 = m3 + m5
    c11 = m4 - m5
    m1 = product(0)
    c22 = (c22 + m1) + product(5)
    c11 = (c11 + m1) + product(6)
    return c11, c12, c21, c22


def _head_major_to_dim_major(val, buf):
    for h in range(H):
        buf[pl.ds(h * PITCH, DH), :] = val[h * DH:(h + 1) * DH]
    return jnp.concatenate([buf[pl.ds(d, H, stride=PITCH), :] for d in range(DH)], axis=0)


def _kernel(x_h, wqkv_h, wo_h, w1_h, w3_h, w2_h, o_h,
            wqkv_in, wo_in, wqkv, wo, w1, w3, w2, w1s, w3s, w2s, xio, xs, xl, hl, tbuf_a, tbuf_b,
            q_s, k_s, v_s, p_s, a_s, sem_x, sem_a, sem_w, sem_o):

    def x_copy(t):
        return pltpu.make_async_copy(x_h.at[pl.ds(t * TM, TM), :], xio.at[t], sem_x.at[t])

    def o_copy(t):
        return pltpu.make_async_copy(xio.at[t], o_h.at[pl.ds(t * TM, TM), :], sem_o.at[t])

    def qkv_copies(n):
        m = n // NR
        cols = pl.ds(pl.multiple_of(m * D, D), D)
        copies = []
        for r0 in (0, HD):
            rows = pl.ds(pl.multiple_of(r0 + (n % NR) * PR, PR), PR)
            copies.append(pltpu.make_async_copy(wqkv_h.at[rows, cols], wqkv_in.at[m, rows, :], sem_a.at[n]))
        return copies

    def wo_copies(j):
        return [pltpu.make_async_copy(wo_h.at[:, pl.ds(pl.multiple_of((j + j0) * 128, 128), 128)],
                                      wo_in.at[j + j0], sem_a.at[3 * NR + j]) for j0 in (0, HB)]

    ffn_copies = [pltpu.make_async_copy(src, dst, sem_w.at[n])
                  for n, (src, dst) in enumerate([(w1_h, w1), (w3_h, w3), (w2_h, w2)])]

    def x_rows(t, j, g0, ng):
        return jnp.concatenate([xs[t, j, pl.ds(g0 + g, 8, stride=XP), :] for g in range(ng)], axis=0)

    def add_to_x(t, j, y):
        for g in range(G):
            xs[t, j, pl.ds(g, 8, stride=XP), :] += y[g * 8:(g + 1) * 8]

    def load_tile(t):
        x_copy(t).wait()
        for j in range(NB):
            val = xio[t, :, j * 128:(j + 1) * 128].astype(F32)
            for s in range(8):
                xs[t, j, pl.ds(s * XP, G), :] = val[s * G:(s + 1) * G]

    def store_tile(t):
        for j in range(NB):
            val = jnp.concatenate([xs[t, j, pl.ds(s * XP, G), :] for s in range(8)], axis=0)
            xio[t, :, j * 128:(j + 1) * 128] = val.astype(BF16)
        o_copy(t).start()

    def normalized(t, g0, ng):
        xb = [x_rows(t, j, g0, ng) for j in range(NB)]
        tot = xb[0]
        for j in range(1, NB):
            tot = tot + xb[j]
        mean = jnp.sum(tot, axis=-1, keepdims=True) * (1.0 / D)
        cb = [b - mean for b in xb]
        sq = cb[0] * cb[0]
        for j in range(1, NB):
            sq = sq + cb[j] * cb[j]
        rstd = lax.rsqrt(jnp.sum(sq, axis=-1, keepdims=True) * (1.0 / D) + 1e-5)
        return [c * rstd for c in cb]

    def layernorm(t, slot, g0):
        top, bot = normalized(t, g0, 2), normalized(t, g0 + G // 2, 2)
        r0 = g0 * 4 if isinstance(g0, int) else pl.multiple_of(g0 * 4, 8)
        for j in range(HB):
            terms = _lhs_terms(top[j], top[j + HB], bot[j], bot[j + HB])
            for i in range(7):
                xl[slot, i, j, pl.ds(r0, 8), :] = _pack(terms[i])

    def next_tile_layernorm(t):
        nt = (t + 1) % NT
        todo = list(range(0, G // 2, 2))

        def step(n):
            for _ in range(min(n, len(todo))):
                layernorm(nt, nt % 2, todo.pop(0))
        return step, todo

    n_steps = 3 * NR
    n_a = n_steps - HB

    def prefetch(n):
        @pl.when(n < n_steps)
        def _():
            for c in qkv_copies(n):
                c.start()

        @pl.when(jnp.logical_and(n >= n_a, n < n_steps))
        def _():
            for c in wo_copies(n - n_a):
                c.start()

    def reorder_qkv_columns(n, buf):
        m = n // NR
        r = pl.multiple_of((n % NR) * PR, PR)
        val = jnp.concatenate([wqkv_in[m, pl.ds(r0 + r, PR), :] for r0 in (0, HD)], axis=0)
        t = pltpu.bitcast(val, U32).T
        val = pltpu.bitcast(_head_major_to_dim_major(t, buf).T, BF16).astype(F32)
        for j in range(HB):
            terms = _rhs_terms(_block(val[:PR], j), _block(val[:PR], j + HB),
                               _block(val[PR:], j), _block(val[PR:], j + HB))
            for i in range(7):
                wqkv[m, i, j, pl.ds(r, PR), :] = terms[i].astype(BF16)

    def prologue_a(i, carry):
        steps = [2 * i, 2 * i + 1]
        for n in steps:
            prefetch(n + AHEAD)
        for n in steps:
            for c in qkv_copies(n):
                c.wait()
        for e, n in enumerate(steps):
            reorder_qkv_columns(n, tbuf_a.at[e])
            layernorm(0, 0, 2 * n)
            k_s[n, pl.ds(TM, HG * 8), :] = jnp.zeros((HG * 8, 128), F32)
            v_s[n, pl.ds(TM, HG * 8), :] = jnp.zeros((HG * 8, 128), F32)
        return carry

    def prologue_b(i, carry):
        steps = [2 * i, 2 * i + 1]
        for n in steps:
            prefetch(n + AHEAD)
        for n in steps:
            for c in qkv_copies(n) + wo_copies(n - n_a):
                c.wait()
        for e, n in enumerate(steps):
            reorder_qkv_columns(n, tbuf_a.at[e])
            j = n - n_a
            left, right = [
                pltpu.bitcast(_head_major_to_dim_major(pltpu.bitcast(wo_in[j + k * HB].astype(F32), U32),
                                                       tbuf_b.at[2 * e + k]), F32) for k in range(2)]
            terms = _rhs_terms(left[:HD], right[:HD], left[HD:], right[HD:])
            for k in range(7):
                wo[k, j] = terms[k].astype(BF16)
        return carry

    assert n_a == NB and 2 * n_a * 2 == G
    x_copy(0).start()
    for n in range(AHEAD):
        for c in qkv_copies(n):
            c.start()
    load_tile(0)
    lax.fori_loop(0, n_a // 2, prologue_a, 0)
    lax.fori_loop(n_a // 2, n_steps // 2, prologue_b, 0)
    for t in range(1, NT):
        x_copy(t).start()
    for c in ffn_copies:
        c.start()

    def project(t, m, j0, j1):
        c11, c12, c21, c22 = _strassen(lambda i: _dot(_wide(xl.at[t % 2, i], 0, HB), _wide(wqkv.at[m, i], j0, j1)))
        for j in range(j0, j1):
            yield j, jnp.concatenate([_block(c11, j - j0), _block(c21, j - j0)], axis=0)
            yield j + HB, jnp.concatenate([_block(c12, j - j0), _block(c22, j - j0)], axis=0)

    def project_with_halo(t, dst, m, j0, j1):
        sub = lax.broadcasted_iota(jnp.int32, (HG * 8, 128), 0) % 8
        for j, new in project(t, m, j0, j1):
            old = dst[j, pl.ds(TM, HG * 8), :]
            prev = jnp.where(t == 0, jnp.broadcast_to(new[0:1, :], (HG * 8, 128)),
                             pltpu.roll(old, HG * 8 - 7, 0))
            dst[j, pl.ds(0, HG * 8), :] = jnp.where(sub == 0, prev, pltpu.roll(new[TM - HG * 8:, :], 1, 0))
            dst[j, pl.ds(HG * 8, TM), :] = new

    def softmax_weights(t, g):
        r = g * 8
        qs = [q_s[j, r:r + 8, :] for j in range(NB)]
        logits = []
        for w in range(W):
            rk = r + (HG - DIL * w) * 8
            a = qs[0] * k_s[0, rk:rk + 8, :]
            for j in range(1, NB):
                a = a + qs[j] * k_s[j, rk:rk + 8, :]
            a = (a + pltpu.roll(a, 64, 1)) + (pltpu.roll(a, 32, 1) + pltpu.roll(a, 96, 1))
            if g < DIL * w:
                pos = t * TM + g + G * lax.broadcasted_iota(jnp.int32, (8, 128), 0)
                a = jnp.where(pos >= DIL * w, a, -1e9 / SCALE)
            logits.append(a)
        mx = logits[0]
        for w in range(1, W):
            mx = jnp.maximum(mx, logits[w])
        ps = [jnp.exp2((a - mx) * (SCALE * LOG2E)) for a in logits]
        den = ps[0]
        for w in range(1, W):
            den = den + ps[w]
        for w in range(W):
            p_s[w, r:r + 8, :] = ps[w]
        p_s[W, r:r + 8, :] = 1.0 / den

    def weighted_values(j):
        def rows(jj, r):
            a = p_s[0, r:r + 16, :] * v_s[jj, r + HG * 8:r + HG * 8 + 16, :]
            for w in range(1, W):
                rk = r + (HG - DIL * w) * 8
                a = a + p_s[w, r:r + 16, :] * v_s[jj, rk:rk + 16, :]
            return a * p_s[W, r:r + 16, :]
        for r in range(0, HM, 16):
            terms = _lhs_terms(rows(j, r), rows(j + HB, r), rows(j, r + HM), rows(j + HB, r + HM))
            for i in range(7):
                a_s[i, j, r // 2:r // 2 + 8, :] = _pack(terms[i])

    def add_quadrants_to_x(t, j0, y):
        for e in range(y[0].shape[1] // 128):
            add_to_x(t, j0 + e, jnp.concatenate([_block(y[0], e), _block(y[2], e)], axis=0))
            add_to_x(t, HB + j0 + e, jnp.concatenate([_block(y[1], e), _block(y[3], e)], axis=0))

    def attention_tile(t, layer):
        @pl.when(jnp.logical_and(layer == 0, t + 1 < NT))
        def _():
            load_tile(t + 1)

        ln_step, ln_todo = next_tile_layernorm(t)
        for j in range(0, HB, 2):
            project_with_halo(t, k_s, 1, j, j + 2)
            ln_step(2)
            for jj, val in project(t, 0, j, j + 2):
                q_s[jj] = val
            ln_step(2)
        assert not ln_todo
        for j in range(HB):
            project_with_halo(t, v_s, 2, j, j + 1)
            for g in range(j * G // HB, (j + 1) * G // HB):
                softmax_weights(t, g)
        for j0 in range(0, HB, 2):
            for j in range(j0, j0 + 2):
                weighted_values(j)
            add_quadrants_to_x(t, 0, _strassen(lambda i: _dot(
                _wide(a_s.at[i], j0, j0 + 2), _wide(wo.at[i, :, j0 * 128:(j0 + 2) * 128, :], 0, HB))))
        return layer

    def ffn_tile(t, layer):
        ln_step, ln_todo = next_tile_layernorm(t)

        def rhs(w, ws, i, n):
            hk, hn = w.shape[0] // 2, w.shape[1] // 2
            if i == 1:
                return w[:hk, n * 128:(n + 2) * 128]
            if i == 4:
                return w[hk:, hn + n * 128:hn + (n + 2) * 128]
            return _wide(ws.at[RHS_SUMS.index(i)], n, n + 2)

        for n in range(0, FB, 2):
            gate = _strassen(lambda i: _dot(_wide(xl.at[t % 2, i], 0, HB), rhs(w1, w1s, i, n)))
            ln_step(1)
            up = _strassen(lambda i: _dot(_wide(xl.at[t % 2, i], 0, HB), rhs(w3, w3s, i, n)))
            if n == FB - 2:
                ln_step(1)
            terms = _lhs_terms(*[g * jax.nn.sigmoid(g) * u for g, u in zip(gate, up)])
            for i in range(7):
                for e in range(2):
                    hl[i, n + e] = _block(terms[i], e).astype(BF16)
        assert not ln_todo
        for n in range(0, HB, 2):
            add_quadrants_to_x(t, n, _strassen(lambda i: _dot(_wide(hl.at[i], 0, FB), rhs(w2, w2s, i, n))))

        @pl.when(layer == N_LAYERS - 1)
        def _():
            store_tile(t)
        return layer

    def run_layer(layer, carry):
        lax.fori_loop(0, NT, attention_tile, layer)

        @pl.when(layer == 0)
        def _():
            for c in ffn_copies:
                c.wait()
            for w, ws in ((w1, w1s), (w3, w3s), (w2, w2s)):
                hk, hn = w.shape[0] // 2, w.shape[1] // 2

                def weight_sums(i, carry, w=w, ws=ws, hk=hk, hn=hn):
                    r = pl.multiple_of(i * 32, 32)
                    for n in range(hn // 128):
                        quads = [w[pl.ds(r0 + r, 32), c0 + n * 128:c0 + (n + 1) * 128].astype(F32)
                                 for r0 in (0, hk) for c0 in (0, hn)]
                        terms = _rhs_terms(*quads)
                        for k, term in enumerate(RHS_SUMS):
                            ws[k, n, pl.ds(r, 32), :] = terms[term].astype(BF16)
                    return carry
                lax.fori_loop(0, hk // 32, weight_sums, 0)
        lax.fori_loop(0, NT, ffn_tile, layer)
        return carry

    lax.fori_loop(0, N_LAYERS, run_layer, 0)
    for t in range(NT):
        o_copy(t).wait()


@jax.jit
def pallas_interleave_layers__sliding_local_dilated__glu_gated_swiglu__prompt_kernel(
    A_x: jax.Array,
    A_wqkv: jax.Array,
    A_wo: jax.Array,
    B_x: jax.Array,
    B_w1: jax.Array,
    B_w3: jax.Array,
    B_w2: jax.Array,
):
    del B_x
    anyspec = pl.BlockSpec(memory_space=pl.ANY)
    out = pl.pallas_call(
        _kernel,
        in_specs=[anyspec] * 6,
        out_specs=anyspec,
        out_shape=jax.ShapeDtypeStruct((S, D), A_x.dtype),
        scratch_shapes=[
            pltpu.VMEM((3, D, D), BF16),
            pltpu.VMEM((NB, D, 128), BF16),
            pltpu.VMEM((3, 7, HB, HD, 128), BF16),
            pltpu.VMEM((7, HB, HD, 128), BF16),
            pltpu.VMEM((D, F), BF16),
            pltpu.VMEM((D, F), BF16),
            pltpu.VMEM((F, D), BF16),
            pltpu.VMEM((5, FB, HD, 128), BF16),
            pltpu.VMEM((5, FB, HD, 128), BF16),
            pltpu.VMEM((5, HB, HF, 128), BF16),
            pltpu.VMEM((NT, TM, D), BF16),
            pltpu.VMEM((NT, NB, 8 * XP + G, 128), F32),
            pltpu.VMEM((2, 7, HB, HM // 2, 128), U32),
            pltpu.VMEM((7, FB, HM, 128), BF16),
            pltpu.VMEM((2, H * PITCH + DH, 128), U32),
            pltpu.VMEM((4, H * PITCH + DH, 128), U32),
            pltpu.VMEM((NB, TM, 128), F32),
            pltpu.VMEM((NB, HG * 8 + TM, 128), F32),
            pltpu.VMEM((NB, HG * 8 + TM, 128), F32),
            pltpu.VMEM((W + 1, TM, 128), F32),
            pltpu.VMEM((7, HB, HM // 2, 128), U32),
            pltpu.SemaphoreType.DMA((NT,)),
            pltpu.SemaphoreType.DMA((3 * NR + HB,)),
            pltpu.SemaphoreType.DMA((3,)),
            pltpu.SemaphoreType.DMA((NT,)),
        ],
        compiler_params=pltpu.CompilerParams(vmem_limit_bytes=116 * 1024 * 1024),
    )(A_x.reshape(S, D), A_wqkv, A_wo, B_w1, B_w3, B_w2)
    return out.reshape(1, S, D)
```

```python
import jax
import jax.numpy as jnp
from jax import lax
import jax.experimental.pallas as pl
import jax.experimental.pallas.tpu as pltpu

S, D, F = 2048, 1024, 3584
H, DH, W, DIL = 32, 32, 8, 2
N_LAYERS = 2
TM = 256
NT = S // TM
G = TM // 8
HG = 16
NB = D // 128
HM, HD, HB = TM // 2, D // 2, NB // 2
HF, FB = F // 2, F // 256
XP = G + 1
PITCH = DH + 1
PR = 128
NR = D // 2 // PR
AHEAD = 4
F32, BF16, U32 = jnp.float32, jnp.bfloat16, jnp.uint32
SCALE = DH ** -0.5
LOG2E = 1.4426950408889634


def _dot(a, b):
    return jnp.dot(a, b, preferred_element_type=F32)


def _wide(ref, j0, j1):
    blocks = [ref[j] for j in range(j0, j1)]
    if ref.dtype == U32:
        blocks = [pltpu.bitcast(b, BF16) for b in blocks]
    return jnp.concatenate(blocks, axis=1)


def _pack(val):
    return pltpu.bitcast(val.astype(BF16), U32)


def _tree_sum(vals):
    while len(vals) > 1:
        vals = [vals[i] + vals[i + 1] for i in range(0, len(vals), 2)]
    return vals[0]


def _silu(x):
    h = 0.5 * x
    return h + h * jnp.tanh(h)


def _block(val, j):
    return val[:, j * 128:(j + 1) * 128]


def _lhs_terms(a11, a12, a21, a22):
    return [a11 + a22, a21 + a22, a11, a22, a11 + a12, a21 - a11, a12 - a22]


def _rhs_terms(b11, b12, b21, b22):
    return [b11 + b22, b11, b12 - b22, b21 - b11, b22, b11 + b12, b21 + b22]


RHS_SUMS = (0, 2, 3, 5, 6)


def _strassen(product):
    m2 = product(1)
    m4 = product(3)
    c21 = m2 + m4
    m3 = product(2)
    c22 = m3 - m2
    m5 = product(4)
    c12 = m3 + m5
    c11 = m4 - m5
    m1 = product(0)
    c22 = (c22 + m1) + product(5)
    c11 = (c11 + m1) + product(6)
    return c11, c12, c21, c22


def _head_major_to_dim_major(val, buf):
    for h in range(H):
        buf[pl.ds(h * PITCH, DH), :] = val[h * DH:(h + 1) * DH]
    return jnp.concatenate([buf[pl.ds(d, H, stride=PITCH), :] for d in range(DH)], axis=0)


def _kernel(x_h, wqkv_h, wo_h, w1_h, w3_h, w2_h, o_h,
            wqkv_in, wo_in, wqkv, wo, w1, w3, w2, w1s, w3s, w2s, xio, xs, xl, hl, tbuf_a, tbuf_b,
            q_s, k_s, v_s, p_s, a_s, sem_x, sem_a, sem_w, sem_o):

    def x_copy(t):
        return pltpu.make_async_copy(x_h.at[pl.ds(t * TM, TM), :], xio.at[t], sem_x.at[t])

    def o_copy(t):
        return pltpu.make_async_copy(xio.at[t], o_h.at[pl.ds(t * TM, TM), :], sem_o.at[t])

    def qkv_copies(n):
        m = n // NR
        cols = pl.ds(pl.multiple_of(m * D, D), D)
        copies = []
        for r0 in (0, HD):
            rows = pl.ds(pl.multiple_of(r0 + (n % NR) * PR, PR), PR)
            copies.append(pltpu.make_async_copy(wqkv_h.at[rows, cols], wqkv_in.at[m, rows, :], sem_a.at[n]))
        return copies

    def wo_copies(j):
        return [pltpu.make_async_copy(wo_h.at[:, pl.ds(pl.multiple_of((j + j0) * 128, 128), 128)],
                                      wo_in.at[j + j0], sem_a.at[3 * NR + j]) for j0 in (0, HB)]

    ffn_copies = [pltpu.make_async_copy(src, dst, sem_w.at[n])
                  for n, (src, dst) in enumerate([(w1_h, w1), (w3_h, w3), (w2_h, w2)])]

    def x_rows(t, j, g0, ng):
        return jnp.concatenate([xs[t, j, pl.ds(g0 + g, 8, stride=XP), :] for g in range(ng)], axis=0)

    def add_to_x(t, j, y):
        for g in range(G):
            xs[t, j, pl.ds(g, 8, stride=XP), :] += y[g * 8:(g + 1) * 8]

    def load_tile(t):
        x_copy(t).wait()
        for j in range(NB):
            val = xio[t, :, j * 128:(j + 1) * 128].astype(F32)
            for s in range(8):
                xs[t, j, pl.ds(s * XP, G), :] = val[s * G:(s + 1) * G]

    def store_tile(t):
        for j in range(NB):
            val = jnp.concatenate([xs[t, j, pl.ds(s * XP, G), :] for s in range(8)], axis=0)
            xio[t, :, j * 128:(j + 1) * 128] = val.astype(BF16)
        o_copy(t).start()

    def normalized(t, g0, ng):
        xb = [x_rows(t, j, g0, ng) for j in range(NB)]
        mean = jnp.sum(_tree_sum(xb), axis=-1, keepdims=True) * (1.0 / D)
        cb = [b - mean for b in xb]
        sq = _tree_sum([c * c for c in cb])
        rstd = lax.rsqrt(jnp.sum(sq, axis=-1, keepdims=True) * (1.0 / D) + 1e-5)
        return [c * rstd for c in cb]

    def layernorm(t, slot, g0):
        top, bot = normalized(t, g0, 2), normalized(t, g0 + G // 2, 2)
        r0 = g0 * 4 if isinstance(g0, int) else pl.multiple_of(g0 * 4, 8)
        for j in range(HB):
            terms = _lhs_terms(top[j], top[j + HB], bot[j], bot[j + HB])
            for i in range(7):
                xl[slot, i, j, pl.ds(r0, 8), :] = _pack(terms[i])

    def next_tile_layernorm(t):
        nt = (t + 1) % NT
        todo = list(range(0, G // 2, 2))

        def step(n):
            for _ in range(min(n, len(todo))):
                layernorm(nt, nt % 2, todo.pop(0))
        return step, todo

    n_steps = 3 * NR
    n_a = n_steps - HB

    def prefetch(n):
        @pl.when(n < n_steps)
        def _():
            for c in qkv_copies(n):
                c.start()

        @pl.when(jnp.logical_and(n >= n_a, n < n_steps))
        def _():
            for c in wo_copies(n - n_a):
                c.start()

    def reorder_qkv_columns(n, buf):
        m = n // NR
        r = pl.multiple_of((n % NR) * PR, PR)
        val = jnp.concatenate([wqkv_in[m, pl.ds(r0 + r, PR), :] for r0 in (0, HD)], axis=0)
        t = pltpu.bitcast(val, U32).T
        val = pltpu.bitcast(_head_major_to_dim_major(t, buf).T, BF16).astype(F32)
        for j in range(HB):
            terms = _rhs_terms(_block(val[:PR], j), _block(val[:PR], j + HB),
                               _block(val[PR:], j), _block(val[PR:], j + HB))
            for i in range(7):
                wqkv[m, i, j, pl.ds(r, PR), :] = terms[i].astype(BF16)

    def prologue_a(i, carry):
        steps = [2 * i, 2 * i + 1]
        for n in steps:
            prefetch(n + AHEAD)
        for n in steps:
            for c in qkv_copies(n):
                c.wait()
        for e, n in enumerate(steps):
            reorder_qkv_columns(n, tbuf_a.at[e])
            layernorm(0, 0, 2 * n)
            k_s[n, pl.ds(TM, HG * 8), :] = jnp.zeros((HG * 8, 128), F32)
            v_s[n, pl.ds(TM, HG * 8), :] = jnp.zeros((HG * 8, 128), F32)
        return carry

    def prologue_b(i, carry):
        steps = [2 * i, 2 * i + 1]
        for n in steps:
            prefetch(n + AHEAD)
        for n in steps:
            for c in qkv_copies(n) + wo_copies(n - n_a):
                c.wait()
        for e, n in enumerate(steps):
            reorder_qkv_columns(n, tbuf_a.at[e])
            j = n - n_a
            left, right = [
                pltpu.bitcast(_head_major_to_dim_major(pltpu.bitcast(wo_in[j + k * HB].astype(F32), U32),
                                                       tbuf_b.at[2 * e + k]), F32) for k in range(2)]
            terms = _rhs_terms(left[:HD], right[:HD], left[HD:], right[HD:])
            for k in range(7):
                wo[k, j] = terms[k].astype(BF16)
        return carry

    assert n_a == NB and 2 * n_a * 2 == G
    x_copy(0).start()
    for c in qkv_copies(0) + qkv_copies(1):
        c.start()
    load_tile(0)
    for n in range(2, AHEAD):
        for c in qkv_copies(n):
            c.start()
    lax.fori_loop(0, n_a // 2, prologue_a, 0)
    lax.fori_loop(n_a // 2, n_steps // 2, prologue_b, 0)
    for t in range(1, NT):
        x_copy(t).start()
    for c in ffn_copies:
        c.start()

    def project(t, m, j0, j1):
        c11, c12, c21, c22 = _strassen(lambda i: _dot(_wide(xl.at[t % 2, i], 0, HB), _wide(wqkv.at[m, i], j0, j1)))
        for j in range(j0, j1):
            yield j, jnp.concatenate([_block(c11, j - j0), _block(c21, j - j0)], axis=0)
            yield j + HB, jnp.concatenate([_block(c12, j - j0), _block(c22, j - j0)], axis=0)

    def project_with_halo(t, dst, m, j0, j1):
        sub = lax.broadcasted_iota(jnp.int32, (HG * 8, 128), 0) % 8
        for j, new in project(t, m, j0, j1):
            old = dst[j, pl.ds(TM, HG * 8), :]
            prev = jnp.where(t == 0, jnp.broadcast_to(new[0:1, :], (HG * 8, 128)),
                             pltpu.roll(old, HG * 8 - 7, 0))
            dst[j, pl.ds(0, HG * 8), :] = jnp.where(sub == 0, prev, pltpu.roll(new[TM - HG * 8:, :], 1, 0))
            dst[j, pl.ds(HG * 8, TM), :] = new

    def softmax_weights(t, g):
        r = g * 8
        qs = [q_s[j, r:r + 8, :] for j in range(NB)]
        logits = []
        for w in range(W):
            rk = r + (HG - DIL * w) * 8
            a = _tree_sum([qs[j] * k_s[j, rk:rk + 8, :] for j in (0, 1, 4, 5, 2, 3, 6, 7)])
            a = (a + pltpu.roll(a, 64, 1)) + (pltpu.roll(a, 32, 1) + pltpu.roll(a, 96, 1))
            if g < DIL * w:
                pos = t * TM + g + G * lax.broadcasted_iota(jnp.int32, (8, 128), 0)
                a = jnp.where(pos >= DIL * w, a, -1e9 / SCALE)
            logits.append(a)
        mx = logits[0]
        for w in range(1, W):
            mx = jnp.maximum(mx, logits[w])
        ps = [jnp.exp2((a - mx) * (SCALE * LOG2E)) for a in logits]
        den = ps[0]
        for w in range(1, W):
            den = den + ps[w]
        for w in range(W):
            p_s[w, r:r + 8, :] = ps[w]
        p_s[W, r:r + 8, :] = 1.0 / den

    def weighted_values(j):
        def rows(jj, r):
            a = _tree_sum([p_s[w, r:r + 16, :] * v_s[jj, pl.ds(r + (HG - DIL * w) * 8, 16), :]
                           for w in range(W)])
            return a * p_s[W, r:r + 16, :]
        for r in range(0, HM, 16):
            terms = _lhs_terms(rows(j, r), rows(j + HB, r), rows(j, r + HM), rows(j + HB, r + HM))
            for i in range(7):
                a_s[i, j, r // 2:r // 2 + 8, :] = _pack(terms[i])

    def add_quadrants_to_x(t, j0, y):
        for e in range(y[0].shape[1] // 128):
            add_to_x(t, j0 + e, jnp.concatenate([_block(y[0], e), _block(y[2], e)], axis=0))
            add_to_x(t, HB + j0 + e, jnp.concatenate([_block(y[1], e), _block(y[3], e)], axis=0))

    def attention_tile(t, layer):
        @pl.when(jnp.logical_and(layer == 0, t + 1 < NT))
        def _():
            load_tile(t + 1)

        ln_step, ln_todo = next_tile_layernorm(t)
        for j in range(0, HB, 2):
            project_with_halo(t, k_s, 1, j, j + 2)
            ln_step(3)
            for jj, val in project(t, 0, j, j + 2):
                q_s[jj] = val
            ln_step(3)
        assert not ln_todo
        for j in range(HB):
            project_with_halo(t, v_s, 2, j, j + 1)
            for g in range(j * G // HB, (j + 1) * G // HB):
                softmax_weights(t, g)
        for j0 in range(0, HB, 2):
            for j in range(j0, j0 + 2):
                weighted_values(j)
            add_quadrants_to_x(t, 0, _strassen(lambda i: _dot(
                _wide(a_s.at[i], j0, j0 + 2), _wide(wo.at[i, :, j0 * 128:(j0 + 2) * 128, :], 0, HB))))
        return layer

    def ffn_tile(t, layer):
        ln_step, ln_todo = next_tile_layernorm(t)

        def rhs(w, ws, i, n):
            hk, hn = w.shape[0] // 2, w.shape[1] // 2
            if i == 1:
                return w[:hk, n * 128:(n + 2) * 128]
            if i == 4:
                return w[hk:, hn + n * 128:hn + (n + 2) * 128]
            return _wide(ws.at[RHS_SUMS.index(i)], n, n + 2)

        for n in range(0, FB, 2):
            gate = _strassen(lambda i: _dot(_wide(xl.at[t % 2, i], 0, HB), rhs(w1, w1s, i, n)))
            ln_step(1)
            up = _strassen(lambda i: _dot(_wide(xl.at[t % 2, i], 0, HB), rhs(w3, w3s, i, n)))
            if n == 0:
                ln_step(1)
            terms = _lhs_terms(*[_silu(g) * u for g, u in zip(gate, up)])
            for i in range(7):
                for e in range(2):
                    hl[i, n + e] = _block(terms[i], e).astype(BF16)
        assert not ln_todo
        for n in range(0, HB, 2):
            add_quadrants_to_x(t, n, _strassen(lambda i: _dot(_wide(hl.at[i], 0, FB), rhs(w2, w2s, i, n))))

        @pl.when(layer == N_LAYERS - 1)
        def _():
            store_tile(t)
        return layer

    def run_layer(layer, carry):
        lax.fori_loop(0, NT, attention_tile, layer)

        @pl.when(layer == 0)
        def _():
            for c in ffn_copies:
                c.wait()
            for w, ws in ((w1, w1s), (w3, w3s), (w2, w2s)):
                hk, hn = w.shape[0] // 2, w.shape[1] // 2

                def weight_sums(i, carry, w=w, ws=ws, hk=hk, hn=hn):
                    r = pl.multiple_of(i * 32, 32)
                    for n in range(hn // 128):
                        quads = [w[pl.ds(r0 + r, 32), c0 + n * 128:c0 + (n + 1) * 128].astype(F32)
                                 for r0 in (0, hk) for c0 in (0, hn)]
                        terms = _rhs_terms(*quads)
                        for k, term in enumerate(RHS_SUMS):
                            ws[k, n, pl.ds(r, 32), :] = terms[term].astype(BF16)
                    return carry
                lax.fori_loop(0, hk // 32, weight_sums, 0)
        lax.fori_loop(0, NT, ffn_tile, layer)
        return carry

    lax.fori_loop(0, N_LAYERS, run_layer, 0)
    for t in range(NT):
        o_copy(t).wait()


@jax.jit
def pallas_interleave_layers__sliding_local_dilated__glu_gated_swiglu__prompt_kernel(
    A_x: jax.Array,
    A_wqkv: jax.Array,
    A_wo: jax.Array,
    B_x: jax.Array,
    B_w1: jax.Array,
    B_w3: jax.Array,
    B_w2: jax.Array,
):
    del B_x
    anyspec = pl.BlockSpec(memory_space=pl.ANY)
    out = pl.pallas_call(
        _kernel,
        in_specs=[anyspec] * 6,
        out_specs=anyspec,
        out_shape=jax.ShapeDtypeStruct((S, D), A_x.dtype),
        scratch_shapes=[
            pltpu.VMEM((3, D, D), BF16),
            pltpu.VMEM((NB, D, 128), BF16),
            pltpu.VMEM((3, 7, HB, HD, 128), BF16),
            pltpu.VMEM((7, HB, HD, 128), BF16),
            pltpu.VMEM((D, F), BF16),
            pltpu.VMEM((D, F), BF16),
            pltpu.VMEM((F, D), BF16),
            pltpu.VMEM((5, FB, HD, 128), BF16),
            pltpu.VMEM((5, FB, HD, 128), BF16),
            pltpu.VMEM((5, HB, HF, 128), BF16),
            pltpu.VMEM((NT, TM, D), BF16),
            pltpu.VMEM((NT, NB, 8 * XP + G, 128), F32),
            pltpu.VMEM((2, 7, HB, HM // 2, 128), U32),
            pltpu.VMEM((7, FB, HM, 128), BF16),
            pltpu.VMEM((2, H * PITCH + DH, 128), U32),
            pltpu.VMEM((4, H * PITCH + DH, 128), U32),
            pltpu.VMEM((NB, TM, 128), F32),
            pltpu.VMEM((NB, HG * 8 + TM, 128), F32),
            pltpu.VMEM((NB, HG * 8 + TM, 128), F32),
            pltpu.VMEM((W + 1, TM, 128), F32),
            pltpu.VMEM((7, HB, HM // 2, 128), U32),
            pltpu.SemaphoreType.DMA((NT,)),
            pltpu.SemaphoreType.DMA((3 * NR + HB,)),
            pltpu.SemaphoreType.DMA((3,)),
            pltpu.SemaphoreType.DMA((NT,)),
        ],
        compiler_params=pltpu.CompilerParams(vmem_limit_bytes=116 * 1024 * 1024),
    )(A_x.reshape(S, D), A_wqkv, A_wo, B_w1, B_w3, B_w2)
    return out.reshape(1, S, D)
```
